```python
import os as _os
_os.environ.setdefault("JAX_PLATFORMS", "cpu")
import jax
import jax.numpy as jnp

def _softmax(x, axis=-1):
    return jax.nn.softmax(x, axis=axis)
def _gelu(x):
    return jax.nn.gelu(x, approximate=True)
def _silu(x):
    return jax.nn.silu(x)
def _sigmoid(x):
    return jax.nn.sigmoid(x)
def _layernorm(x, axis=-1, eps=1e-5):
    m = jnp.mean(x, axis=axis, keepdims=True)
    v = jnp.var(x, axis=axis, keepdims=True)
    return (x - m) / jnp.sqrt(v + eps)
def _scatter_add(tgt, idx, src, axis=0):
    return tgt.at[idx].add(src)
def _segment_sum(src, seg, n):
    return jax.ops.segment_sum(src, seg, n)
class _Rng:
    def __init__(self, key):
        self._k = key
    def _next(self):
        self._k, sub = jax.random.split(self._k)
        return sub
    def normal(self, shape):
        return jax.random.normal(self._next(), shape, dtype=jnp.bfloat16)
    def randint(self, lo, hi, shape):
        return jax.random.randint(self._next(), shape, lo, hi, dtype=jnp.int32)
    def uniform(self, shape, lo=0.0, hi=1.0):
        return jax.random.uniform(self._next(), shape, jnp.bfloat16, lo, hi)
    def permutation(self, n):
        return jax.random.permutation(self._next(), n)


kernel_name = 'gated_mix__ssm_conv_h3__mixer_s_mlp__prompt'

def setup_inputs():
    _rng = _Rng(jax.random.key(int.from_bytes(__import__("os").urandom(4), "little")))
    _w = (lambda a: (lambda t: t.astype(jnp.bfloat16) if jnp.issubdtype(t.dtype, jnp.floating) else t)(jnp.asarray(a)))
    def _A_setup():
        B, S, D = 1, 2048, 576
        ks = 4
        return {
            "q": _w((lambda *s: _rng.normal(s) * 0.05)(B, S, D)),
            "k": _w((lambda *s: _rng.normal(s) * 0.4)(B, S, D)),
            "v": _w((lambda *s: _rng.normal(s) * 0.4)(B, S, D)),
            "shift_k": _w((lambda *s: _rng.normal(s) * 0.4)(D, ks) * 0.5),
            "ssm_k": _w((lambda *s: _rng.normal(s) * 0.4)(D, S) * (1.0 / S ** 0.5)),
            "ssm_D": _w((lambda *s: _rng.normal(s) * 0.4)(D)),
        }
    _A_in = _A_setup()

    def _B_setup():
        B, S, D, F = 1, 2048, 576, 4608
        return {
            "x":  _w((lambda *s: _rng.normal(s) * 0.05)(B, S, D)),
            "w1": _w((lambda *s: _rng.normal(s) * 0.2)(D, D) * (D ** -0.5)),
            "w2": _w((lambda *s: _rng.normal(s) * 0.2)(D, D) * (D ** -0.5)),
            "w3": _w((lambda *s: _rng.normal(s) * 0.2)(D, F) * (D ** -0.5)),
            "w4": _w((lambda *s: _rng.normal(s) * 0.2)(F, D) * (F ** -0.5)),
        }
    _B_in = _B_setup()

    return {
        "A_q": _A_in["q"],
        "A_k": _A_in["k"],
        "A_v": _A_in["v"],
        "A_shift_k": _A_in["shift_k"],
        "A_ssm_k": _A_in["ssm_k"],
        "A_ssm_D": _A_in["ssm_D"],
        "B_x": _B_in["x"],
        "B_w1": _B_in["w1"],
        "B_w2": _B_in["w2"],
        "B_w3": _B_in["w3"],
        "B_w4": _B_in["w4"],
        "gate_w": _w((lambda *s: _rng.normal(s) * 0.05)(576) * 16.0),
    }

def reference(A_q, A_k, A_v, A_shift_k, A_ssm_k, A_ssm_D, B_x, B_w1, B_w2, B_w3, B_w4, gate_w):
    def _A_ref(q, k, v, shift_k, ssm_k, ssm_D):
        B, S, D = q.shape
        ks = shift_k.shape[-1]
        k_pad = jnp.pad(k, ((0, 0), (ks - 1, 0), (0, 0)))
        k_shift = jnp.zeros_like(k)
        for t in range(ks):
            k_shift = k_shift + k_pad[:, t:t + S, :] * shift_k[:, ks - 1 - t][None, None, :]
        kv = k_shift * v
        L = 2 * S
        kv_pad = jnp.pad(kv, ((0, 0), (0, S), (0, 0)))
        kf_pad = jnp.pad(ssm_k, ((0, 0), (0, S)))
        kv_f = (lambda x, axes=(-2,-1): jnp.fft.rfft2(x.astype(jnp.float32), axes=axes))(kv_pad[:, None, :, :], axes=(1, 2))
        kf_f = (lambda x, axes=(-2,-1): jnp.fft.rfft2(x.astype(jnp.float32), axes=axes))(kf_pad[:, None, :], axes=(1, 2))
        kf_f = (lambda x, *d: x.transpose(*d))(kf_f, 1, 2, 0)
        y_f = kv_f * kf_f[None, :, :, :]
        y = (lambda x, s, axes=(-2,-1): jnp.fft.irfft2(x, s=s, axes=axes).astype(jnp.bfloat16))(y_f, (1, L), axes=(1, 2))[:, 0, :S, :]
        y = y + kv * ssm_D[None, None, :]
        return q * y

    def _B_ref(x, w1, w2, w3, w4):
        B, S, D = x.shape
        h = _gelu(_layernorm(x, axis=-1) @ w1)
        c = D // 4
        g0 = jnp.pad(h[:, :, 0*c:1*c], ((0, 0), (1, 0), (0, 0)))[:, :S, :]
        g1 = jnp.pad(h[:, :, 1*c:2*c], ((0, 0), (0, 1), (0, 0)))[:, 1:, :]
        g2 = jnp.pad(h[:, :, 2*c:3*c], ((0, 0), (2, 0), (0, 0)))[:, :S, :]
        g3 = jnp.pad(h[:, :, 3*c:   ], ((0, 0), (0, 2), (0, 0)))[:, 2:, :]
        hs = jnp.concatenate([g0, g1, g2, g3], axis=-1) @ w2
        x1 = x + hs
        h2 = _gelu(_layernorm(x1, axis=-1) @ w3) @ w4
        return x1 + h2

    x = A_q
    g = _sigmoid((x * gate_w).sum(-1, keepdims=True))
    a = _A_ref(x, A_k, A_v, A_shift_k, A_ssm_k, A_ssm_D)
    b = _B_ref(x, B_w1, B_w2, B_w3, B_w4)
    return g * a + (1 - g) * b
```

```python
import functools

import numpy as np
import jax
import jax.numpy as jnp
from jax import lax
import jax.experimental.pallas as pl
import jax.experimental.pallas.tpu as pltpu

BF = jnp.bfloat16
F32 = jnp.float32

S, D, F = 2048, 576, 4608
KS = 4
Q = 128
NC = S // Q
TP = 4 * Q
NP = S // TP
FC = 4 * Q
NJ = F // FC
G = D // NJ
DQ = D // 4
EPS = 1e-5

_C0 = float(np.sqrt(2.0 / np.pi))
SC = float((_C0 * 0.044715) ** (1.0 / 3.0))
AA = _C0 / SC
UNSC = 0.5 / SC

CFG = dict(tb1=512, lag=1, peel0=False)


def _dft_matrices():
    theta = 2.0 * np.pi * (np.arange(Q) + 0.25) / Q
    ang = np.arange(Q)[:, None] * theta[None, :]
    fwd = np.concatenate([np.cos(ang), -np.sin(ang)], axis=1)
    inv = np.concatenate([np.cos(ang).T, -np.sin(ang).T], axis=0) / Q
    return fwd.astype(np.float32), inv.astype(np.float32)


_FWD, _INV = _dft_matrices()


def _dot(a, b):
    return jnp.dot(a, b, preferred_element_type=F32)


def _dot_nt(a, b):
    return lax.dot_general(a, b, (((1,), (1,)), ((), ())), preferred_element_type=F32)


def _gelu2(xs):
    return xs * jnp.tanh(xs * (xs * xs + AA)) + xs


def _ln_scaled(x):
    xc = x - jnp.sum(x, axis=0, keepdims=True) * (1.0 / D)
    var = jnp.sum(xc * xc, axis=0, keepdims=True) * (1.0 / D)
    return xc * (lax.rsqrt(var + EPS) * SC)


K2 = ((0, 0), (0, 1), (1, 0), (1, 1))
UP_ORDER = (2, 4, 1, 3, 0, 6, 5)
DN_ORDER = (1, 0, 4, 3, 6, 2, 5)


def _enc_a(a):
    return [a[0, 0] + a[1, 1], a[1, 0] + a[1, 1], a[0, 0], a[1, 1],
            a[0, 0] + a[0, 1], a[1, 0] - a[0, 0], a[0, 1] - a[1, 1]]


def _enc_b(b):
    return [b[0, 0] + b[1, 1], b[0, 0], b[0, 1] - b[1, 1], b[1, 0] - b[0, 0],
            b[1, 1], b[0, 0] + b[0, 1], b[1, 0] + b[1, 1]]


def _dec(m):
    return {(0, 1): m[2] + m[4], (1, 0): m[1] + m[3],
            (0, 0): (m[3] - m[4]) + m[0] + m[6], (1, 1): (m[2] - m[1]) + m[0] + m[5]}


def _enc2(enc, blk):
    outer = {k: enc({(r, c): blk[2 * r + k[0]][2 * c + k[1]] for r, c in K2}) for k in K2}
    return [t for i in range(7) for t in enc({k: outer[k][i] for k in K2})]


def _dec2(m):
    inner = [_dec(m[7 * i:7 * i + 7]) for i in range(7)]
    out = {}
    for k in K2:
        for (r, c), v in _dec([inner[i][k] for i in range(7)]).items():
            out[2 * r + k[0], 2 * c + k[1]] = v
    return out


def _comb(f, *ds):
    return {k: f(*[d[k] for d in ds]) for k in K2}


def _causal_conv(a, b):
    out = []
    for c in range(len(a)):
        acc = a[0] * b[c]
        for m in range(1, c + 1):
            acc = acc + a[m] * b[c - m]
        out.append(acc)
    return out


def _kernel(shift_ref, ssmd_ref, gate_ref, fwd_ref, inv_ref,
            x_hbm, k_hbm, v_hbm, s_hbm, w1_hbm, w2_hbm, w3_hbm, w4_hbm,
            o_hbm,
            kb, vb, sb, xb, w1b, w2b, w3b, w4b, w1t, w2t, coef, x1b, xa, xr,
            w3c, w4c, acc, yb, gqb, gsb, ob,
            sem_x, sem_w, sem_k, sem_v, sem_s, sem_w3, sem_w4, sem_o):

    def x_copy(p):
        sl = pl.ds(p * TP, TP)
        return pltpu.make_async_copy(x_hbm.at[:, sl], xb.at[:, sl], sem_x.at[p])

    def o_copy(p):
        sl = pl.ds(p * TP, TP)
        return pltpu.make_async_copy(ob.at[:, sl], o_hbm.at[:, sl], sem_o.at[p])

    w1_copy = pltpu.make_async_copy(w1_hbm, w1b, sem_w.at[0])
    w2_copy = pltpu.make_async_copy(w2_hbm, w2b, sem_w.at[1])

    def conv_copies(j):
        rows = pl.ds(pl.multiple_of(j * G, G), G)
        return [pltpu.make_async_copy(h.at[rows, :], b.at[rows, :], s.at[j])
                for h, b, s in ((k_hbm, kb, sem_k), (v_hbm, vb, sem_v), (s_hbm, sb, sem_s))]

    def mlp_copies(j):
        cols = pl.ds(pl.multiple_of(j * FC, FC), FC)
        return [pltpu.make_async_copy(h.at[:, cols], b.at[:, cols], s.at[j])
                for h, b, s in ((w3_hbm, w3b, sem_w3), (w4_hbm, w4b, sem_w4))]

    def start(copies):
        for c in copies:
            c.start()

    def wait(copies):
        for c in copies:
            c.wait()

    lane = lax.broadcasted_iota(jnp.int32, (1, Q), 1)

    def prep_weights(j):
        c0 = j * FC
        col = lambda h: pl.ds(pl.multiple_of(c0 + h * Q, Q), Q)
        b = [[w3b[k * Q:(k + 1) * Q, col(h)].astype(F32) for h in range(4)] for k in range(4)]
        for i, t in enumerate(_enc2(_enc_b, b)):
            w3c[j, i] = t.astype(BF)
        a = [[w4b[f * DQ:(f + 1) * DQ, col(3 - k)].astype(F32) for k in range(4)] for f in range(4)]
        for i, t in enumerate(_enc2(_enc_a, a)):
            w4c[j, i] = t.astype(BF)

    def conv_thunks(j):
        thunks = []
        for u in range(G // 16):
            r0 = pl.multiple_of(j * G + 16 * u, 16)
            st = {}

            def load(r0=r0, st=st):
                rows = pl.ds(r0, 16)
                k16 = kb[rows, :].astype(F32)
                v16 = vb[rows, :].astype(F32)
                s16 = sb[rows, :].astype(F32)
                taps = [coef[t, rows, :] for t in range(KS)]
                prev = [jnp.zeros((16, Q), F32)] * KS
                kv, ker = [], []
                for c in range(NC):
                    kc = k16[:, c * Q:(c + 1) * Q]
                    cur = [kc] + [pltpu.roll(kc, t, 1) for t in range(1, KS)]
                    ks = kc * taps[0]
                    for t in range(1, KS):
                        ks = ks + jnp.where(lane >= t, cur[t], prev[t]) * taps[t]
                    prev = cur
                    kv.append(ks * v16[:, c * Q:(c + 1) * Q])
                    ker.append(s16[:, c * Q:(c + 1) * Q])
                ker[0] = ker[0] + jnp.where(lane == 0, coef[KS, rows, :], 0.0)
                st['kv'], st['ker'] = kv, ker

            for hf in range(2):
                def forward(hf=hf, st=st, load=load):
                    if hf == 0:
                        load()
                    sl = slice(8 * hf, 8 * hf + 8)
                    lhs = jnp.concatenate(
                        [t for c in range(NC) for t in (st['kv'][c][sl], st['ker'][c][sl])], axis=0)
                    t = _dot(lhs.astype(BF), fwd_ref[...])
                    ur = [t[16 * c:16 * c + 8, :Q] for c in range(NC)]
                    ui = [t[16 * c:16 * c + 8, Q:] for c in range(NC)]
                    kr = [t[16 * c + 8:16 * c + 16, :Q] for c in range(NC)]
                    ki = [t[16 * c + 8:16 * c + 16, Q:] for c in range(NC)]
                    a = [kr[0]] + [kr[m] - ki[m - 1] for m in range(1, NC)]
                    b = [ki[0]] + [ki[m] + kr[m - 1] for m in range(1, NC)]
                    s1 = _causal_conv([x + y for x, y in zip(a, b)], ur)
                    s2 = _causal_conv(a, [y - x for x, y in zip(ur, ui)])
                    s3 = _causal_conv(b, [x + y for x, y in zip(ur, ui)])
                    zr = jnp.concatenate([x - y for x, y in zip(s1, s3)], axis=0)
                    zi = jnp.concatenate([x + y for x, y in zip(s1, s2)], axis=0)
                    st['z', hf] = jnp.concatenate([zr, zi], axis=1).astype(BF)

                def inverse(hf=hf, st=st, r0=r0):
                    y = _dot(st['z', hf], inv_ref[...])
                    rows = pl.ds(pl.multiple_of(r0 + 8 * hf, 8), 8)
                    for c in range(NC):
                        yb[rows, c * Q:(c + 1) * Q] = y[8 * c:8 * c + 8]

                thunks.append((forward, inverse))

        return thunks

    def mlp_stages(j, mode):
        ups, dns = [], []
        for p in range(NP):
            st = {}

            def rprod(t, h, p=p):
                r = _dot(xr[p * TP + t * 2 * Q:p * TP + (t + 1) * 2 * Q, :],
                         w3b[4 * Q:D, pl.ds(pl.multiple_of(j * FC + h * 2 * Q, 2 * Q), 2 * Q)])
                return {(a, b): r[a * Q:(a + 1) * Q, b * Q:(b + 1) * Q] for a, b in K2}

            def group(o, p=p):
                m = [None] * 7
                for i in UP_ORDER:
                    m[i] = _dot(xa[7 * o + i, p * Q:(p + 1) * Q, :], w3c[j, 7 * o + i])
                return _dec(m)

            def enc(b):
                return [t.astype(BF) for t in _enc_b({(k, n): b[n, 1 - k] for k, n in K2})]

            def s0(st=st, rprod=rprod, group=group):
                r = rprod(0, 1)
                st['m2'], st['m4'] = group(2), group(4)
                st['b00'] = _comb(lambda r, a, b: _gelu2(r + a + b), r, st['m2'], st['m4'])
                st[1] = enc(st['b00'])

            def s1(st=st, rprod=rprod, group=group):
                r = rprod(1, 0)
                st['m1'], st['m3'] = group(1), group(3)
                st['b11'] = _comb(lambda r, a, b: _gelu2(r + a + b), r, st['m1'], st['m3'])
                st[0] = enc(_comb(lambda a, b: a + b, st['b00'], st['b11']))
                st[4] = enc(st['b11'])

            def s2(st=st, rprod=rprod, group=group):
                t = _comb(lambda r, a, b: r + (a - b), rprod(0, 0), st['m3'], st['m4'])
                st['m0'] = group(0)
                b10 = _comb(lambda t, a, b: _gelu2(t + a + b), t, st['m0'], group(6))
                st[3] = enc(_comb(lambda a, b: a - b, b10, st['b00']))
                st[6] = enc(_comb(lambda a, b: a + b, b10, st['b11']))

            def s3(st=st, rprod=rprod, group=group):
                t = _comb(lambda r, a, b, c: r + (a - b) + c, rprod(1, 1), st['m2'], st['m1'], st['m0'])
                b01 = _comb(lambda t, a: _gelu2(t + a), t, group(5))
                st[2] = enc(_comb(lambda a, b: a - b, b01, st['b11']))
                st[5] = enc(_comb(lambda a, b: a + b, st['b00'], b01))

            def down(groups, p=p, st=st):
                for o in groups:
                    for i in DN_ORDER:
                        n = 7 * o + i
                        d = _dot_nt(w4c[j, n], st[o][i])
                        cols = slice(p * Q, (p + 1) * Q)
                        if mode == 'first':
                            acc[n, :, cols] = d
                        elif mode == 'mid':
                            acc[n, :, cols] += d
                        else:
                            st['out', n] = acc[n, :, cols] + d
                if mode == 'last' and groups[-1] == DN_ORDER[-1]:
                    epilogue(p, [st['out', n] for n in range(49)])

            ups += [s0, s1, s2, s3]
            dns += [functools.partial(down, g) for g in ((1,), (0, 4), (3, 6), (2, 5))]
        return ups, dns

    def epilogue(p, m):
        for (f, n), o in _dec2(m).items():
            rows = slice(f * DQ, (f + 1) * DQ)
            cols = slice(p * TP + n * Q, p * TP + (n + 1) * Q)
            base = gqb[rows, cols] * yb[rows, cols] + x1b[rows, cols]
            ob[rows, cols] = (base + o * gsb[0:1, cols]).astype(BF)
        o_copy(p).start()

    def step(j, mode):
        ups, dns = mlp_stages(j, mode)
        lag = CFG['lag']
        n = len(ups) + lag
        extra = [[] for _ in range(n)]
        if mode != 'last':
            prep_weights(j + 1)
            for i, (fw, iv) in enumerate(conv_thunks(j + 1)):
                extra[2 * i].append(fw)
                extra[min(2 * i + 2, n - 1)].append(iv)
        for s in range(n):
            for t in extra[s]:
                t()
            if s < len(ups):
                ups[s]()
            if s >= lag:
                dns[s - lag]()

    x_copy(0).start()
    w1_copy.start()
    start(conv_copies(0))
    x_copy(1).start()
    w2_copy.start()
    x_copy(2).start()
    x_copy(3).start()
    start(mlp_copies(0))
    start(conv_copies(1))
    start(mlp_copies(1))

    sh = shift_ref[...].astype(F32)
    vecs = [sh[t:t + 1] for t in range(KS)]
    vecs += [r[...].astype(F32).reshape(1, D) for r in (ssmd_ref, gate_ref)]
    for i, r in enumerate(vecs):
        coef[i] = jnp.broadcast_to(r, (Q, D)).T

    tb = CFG['tb1']
    nb = S // tb
    cpb = tb // Q
    hc = [None] * NC
    gate = [None] * nb
    xn2 = [None] * NC
    zero = jnp.zeros((DQ, Q), F32)

    def stage1(b):
        if (b * tb) % TP == 0:
            x_copy(b * tb // TP).wait()
        cols = slice(b * tb, (b + 1) * tb)
        x = xb[:, cols].astype(F32)
        xn = _ln_scaled(x).astype(BF)
        gw = coef[KS + 1]
        z = jnp.sum(x * jnp.concatenate([gw] * cpb, axis=1), axis=0, keepdims=True)
        g = 1.0 / (1.0 + jnp.exp(-z))
        gate[b] = g
        gqb[:, cols] = g * x
        gsb[:, cols] = jnp.broadcast_to((1.0 - g) * UNSC, (8, tb))
        if b == 0:
            w1_copy.wait()
            w1t[...] = w1b[...].astype(F32).T.astype(BF)
        h = _gelu2(_dot(w1t[...], xn))
        for i in range(cpb):
            t = h[:, i * Q:(i + 1) * Q]
            hc[b * cpb + i] = [pltpu.roll(t[g * DQ:(g + 1) * DQ], sft, 1)
                               for g, sft in enumerate((1, Q - 1, 2, Q - 2))]

    def shifted(c):
        lo = hc[c - 1] if c > 0 else [zero] * 4
        hi = hc[c + 1] if c + 1 < NC else [zero] * 4
        cur = hc[c]
        return jnp.concatenate([jnp.where(lane >= 1, cur[0], lo[0]),
                                jnp.where(lane < Q - 1, cur[1], hi[1]),
                                jnp.where(lane >= 2, cur[2], lo[2]),
                                jnp.where(lane < Q - 2, cur[3], hi[3])], axis=0)

    def stage2(b):
        if b == 0:
            w2_copy.wait()
            w2t[...] = w2b[...].astype(F32).T.astype(BF)
        hs = jnp.concatenate([shifted(b * cpb + i) for i in range(cpb)], axis=1).astype(BF)
        cols = slice(b * tb, (b + 1) * tb)
        x1 = xb[:, cols].astype(F32) + _dot(w2t[...], hs) * UNSC
        x1b[:, cols] = (1.0 - gate[b]) * x1
        xn = _ln_scaled(x1)
        for i in range(cpb):
            xn2[b * cpb + i] = xn[:, i * Q:(i + 1) * Q].T
        if ((b + 1) * tb) % TP == 0:
            p = (b + 1) * tb // TP - 1
            blk = [[xn2[4 * p + t][:, k * Q:(k + 1) * Q] for k in range(4)] for t in range(4)]
            for i, t in enumerate(_enc2(_enc_a, blk)):
                xa[i, p * Q:(p + 1) * Q, :] = t.astype(BF)
            for t in range(4):
                xr[p * TP + t * Q:p * TP + (t + 1) * Q, :] = xn2[4 * p + t][:, 4 * Q:].astype(BF)

    for b in range(nb + 1):
        if b < nb:
            stage1(b)
        if b == 0:
            wait(conv_copies(0))
            pending = [t for pair in conv_thunks(0) for t in pair]
        take = -(-len(pending) // (nb + 1 - b))
        for t in pending[:take]:
            t()
        pending = pending[take:]
        if b >= 1:
            stage2(b - 1)
    wait(mlp_copies(0))
    prep_weights(0)

    def fetch(j):
        wait(conv_copies(j + 1))
        wait(mlp_copies(j + 1))

    def body(j, carry):
        @pl.when(j + 2 < NJ)
        def _():
            start(conv_copies(j + 2))
            start(mlp_copies(j + 2))
        fetch(j)
        step(j, 'mid')
        return carry

    start(conv_copies(2))
    start(mlp_copies(2))
    fetch(0)
    step(0, 'first')
    lax.fori_loop(1, NJ - 1, body, 0)
    step(NJ - 1, 'last')
    for p in range(NP):
        o_copy(p).wait()


@jax.jit
def pallas_gated_mix__ssm_conv_h3__mixer_s_mlp__prompt_kernel(
    A_q: jax.Array,
    A_k: jax.Array,
    A_v: jax.Array,
    A_shift_k: jax.Array,
    A_ssm_k: jax.Array,
    A_ssm_D: jax.Array,
    B_x: jax.Array,
    B_w1: jax.Array,
    B_w2: jax.Array,
    B_w3: jax.Array,
    B_w4: jax.Array,
    gate_w: jax.Array,
):
    t = lambda a: a.reshape(S, D).T
    vmem = pl.BlockSpec(memory_space=pltpu.VMEM)
    hbm = pl.BlockSpec(memory_space=pl.ANY)
    dma = pltpu.SemaphoreType.DMA
    scratch = (
        [pltpu.VMEM((D, S), BF)] * 4
        + [pltpu.VMEM((D, D), BF)] * 2
        + [pltpu.VMEM((D, F), BF)] * 2
        + [pltpu.VMEM((D, D), BF)] * 2
        + [pltpu.VMEM((KS + 2, D, Q), F32),
           pltpu.VMEM((D, S), F32),
           pltpu.VMEM((49, S // 4, Q), BF),
           pltpu.VMEM((S, D - 4 * Q), BF),
           pltpu.VMEM((NJ, 49, Q, Q), BF),
           pltpu.VMEM((NJ, 49, DQ, Q), BF),
           pltpu.VMEM((49, DQ, S // 4), F32),
           pltpu.VMEM((D, S), F32),
           pltpu.VMEM((D, S), F32),
           pltpu.VMEM((8, S), F32),
           pltpu.VMEM((D, S), BF)]
        + [dma((NP,)), dma((2,))] + [dma((NJ,))] * 5 + [dma((NP,))]
    )
    out_t = pl.pallas_call(
        _kernel,
        in_specs=[vmem] * 5 + [hbm] * 8,
        out_specs=hbm,
        out_shape=jax.ShapeDtypeStruct((D, S), BF),
        scratch_shapes=scratch,
        compiler_params=pltpu.CompilerParams(vmem_limit_bytes=120 * 1024 * 1024),
    )(A_shift_k.T, A_ssm_D, gate_w, jnp.asarray(_FWD, BF), jnp.asarray(_INV, BF),
      t(A_q), t(A_k), t(A_v), A_ssm_k, B_w1, B_w2, B_w3, B_w4.T)
    return out_t.T.reshape(1, S, D)
```

```python
import collections
import functools

import numpy as np
import jax
import jax.numpy as jnp
from jax import lax
import jax.experimental.pallas as pl
import jax.experimental.pallas.tpu as pltpu

BF = jnp.bfloat16
F32 = jnp.float32
I32 = jnp.int32

S, D, F = 2048, 576, 4608
KS = 4
Q = 128
NC = S // Q
TP = 4 * Q
NP = S // TP
FC = 4 * Q
NJ = F // FC
KD = 3
DQ = D // 4
DR = D - 4 * Q
TB = 2 * Q
NG = D // 8
EPS = 1e-5
N_SEMS = 34

_C0 = float(np.sqrt(2.0 / np.pi))
SC = float((_C0 * 0.044715) ** (1.0 / 3.0))
AA = _C0 / SC
UNSC = 0.5 / SC


def _bf16_words(a):
    u = a.astype(np.float32).view(np.uint32)
    u = (u + 0x7FFF + ((u >> 16) & 1)) >> 16
    return (u[0::2] | (u[1::2] << 16)).astype(np.uint32).view(np.int32)


def _transform_matrices():
    theta = 2.0 * np.pi * (np.arange(Q) + 0.25) / Q
    ang = np.arange(Q)[:, None] * theta[None, :]
    fwd = np.concatenate([np.cos(ang), -np.sin(ang)], axis=1)
    inv = np.concatenate([np.cos(ang).T, -np.sin(ang).T], axis=0) / Q
    return _bf16_words(fwd), _bf16_words(inv)


_FWD, _INV = _transform_matrices()
assert (_INV[0:8] != 0).all()


def _gelu(xs):
    return xs * jnp.tanh(xs * (xs * xs + AA)) + xs


def _layernorm(x):
    mean = jnp.sum(x, axis=0, keepdims=True) * (1.0 / D)
    xc = x - mean
    var = jnp.sum(xc * xc, axis=0, keepdims=True) * (1.0 / D)
    scale = lax.rsqrt(var + EPS) * SC
    return x * scale - mean * scale


K2 = ((0, 0), (0, 1), (1, 0), (1, 1))
WIDE = (0, 3, 4, 6)


def _enc_a(a):
    return [a[0, 0] + a[1, 1], a[1, 0] + a[1, 1], a[0, 0], a[1, 1],
            a[0, 0] + a[0, 1], a[1, 0] - a[0, 0], a[0, 1] - a[1, 1]]


def _enc_b(b):
    return [b[0, 0] + b[1, 1], b[0, 0], b[0, 1] - b[1, 1], b[1, 0] - b[0, 0],
            b[1, 1], b[0, 0] + b[0, 1], b[1, 0] + b[1, 1]]


_TERM_A = ((0, 0), (1, 0), (0, 0), (1, 1), (0, 0), (1, 0), (0, 1))
_TERM_B = ((0, 0), (0, 0), (0, 1), (1, 0), (1, 1), (0, 0), (1, 0))


def _wide_a(a0, a1):
    return [a1, a1, a0, a0 - a1]


def _wide_b(b0, b1):
    return [b1, b0, b1, b0 + b1]


def _wide2(enc, quarters):
    outer = [enc(quarters[k], quarters[2 + k]) for k in range(2)]
    return [t for o in range(4) for t in enc(outer[0][o], outer[1][o])]


def _two(a, b):
    return a + b


def _four(a, b, c, d):
    return (a - b) + c + d


DECODE = (((0, 1), (2, 4), _two), ((1, 0), (1, 3), _two),
          ((0, 0), (3, 4, 0, 6), _four), ((1, 1), (2, 1, 0, 5), _four))


def _dec(m):
    return {blk: fn(*(m[i] for i in terms)) for blk, terms, fn in DECODE}


def _blockwise(fn, *ds):
    return {k: fn(*(d[k] for d in ds)) for k in K2}


STAGE_GROUPS = ((2, 4), (1, 3), (0, 6), (5,))
STAGE_ORDER = {
    1: ((0, 2), (0, 4), (0, 1), (0, 3), (0, 0), None, (0, 6), None, (0, 5), None, None),
    2: ((0, 1), (0, 2), (0, 4), None, (0, 3), (1, 3), (1, 2), (1, 4), (1, 1), None,
        (0, 0), (0, 6), (0, 5), None, (1, 0), (1, 6), None, (1, 5)),
}
DOWN_ORDER = (1, 0, 4, 3, 6, 2, 5)
DOWN_READY = {1: 0, 0: 1, 4: 1, 3: 2, 6: 2, 2: 3, 5: 3}
DOWN_LAG = 4
HEAD = 'n2 n3 f2 n4 f3 f4 x0 s0 n5 n6 n7 s1 s2 f5 f6 f7 w0 s3 s4 s5 s6 s7'
MATMUL = 1000
MATMUL_TICKS = ((2, 6), (0, 4), (0, 4), (2, 6))
CONV_PAUSES = (1, 2, 2)
LAST_INPUTS_TICK = 175
RATES = dict(x=1.4, w=2.3, early=0.33, late=0.2)
MAX_CREDIT = 200


def _kernel(shift_hbm, ssmd_hbm, gate_hbm, fwd_hbm, inv_hbm,
            x_hbm, k_hbm, v_hbm, s_hbm, w1_hbm, w2_hbm, w3_hbm, w4_hbm,
            o_hbm,
            shift_ref, ssmd_ref, gate_ref, fwd_ref, inv_ref,
            kb, vb, sb, xb, w1b, w2b, w3b, w4b, xa, xr, w3a, w3r, w4a, coef, x1b, yb, gb, ob,
            sem):
    P = functools.partial

    sems = iter(range(N_SEMS))

    def copy(src, dst, rows=(0, D), cols=None):
        if cols is not None:
            at = (pl.ds(rows[0], rows[1] - rows[0]), pl.ds(cols[0], cols[1] - cols[0]))
            src, dst = src.at[at], dst.at[at]
        return pltpu.make_async_copy(src, dst, sem.at[next(sems)])

    def start(*copies):
        for c in copies:
            c.start()

    def wait(*copies):
        for c in copies:
            c.wait()

    small_in = [copy(shift_hbm, shift_ref), copy(ssmd_hbm, ssmd_ref), copy(gate_hbm, gate_ref),
                copy(inv_hbm, inv_ref)]
    x_in = [copy(x_hbm, xb, cols=c) for c in ((0, 2 * TB), (2 * TB, 5 * TB), (5 * TB, S))]
    w1_in, w2_in = copy(w1_hbm, w1b), copy(w2_hbm, w2b)
    w3_in = [copy(w3_hbm, w3b, cols=c) for c in ((0, 2 * FC), (2 * FC, KD * FC), (KD * FC, F))]
    w4_in = [copy(w4_hbm, w4b, cols=c) for c in ((0, KD * FC), (KD * FC, F))]
    conv_in = [copy(fwd_hbm, fwd_ref), copy(k_hbm, kb), copy(v_hbm, vb), copy(s_hbm, sb)]
    out_copy = {(p, f, t): copy(ob, o_hbm, (f * 2 * DQ, (f + 1) * 2 * DQ),
                                (p * TP + t * 2 * Q, p * TP + (t + 1) * 2 * Q))
                for p in range(NP) for f, t in K2}

    last = [None]
    done = set()
    background = collections.deque()
    credit = dict(left=0.0, rate=0.0)

    def release(d):
        last[0] = d
        for r in range(0, d.shape[0], 32):
            credit['left'] = min(credit['left'] + 32 * credit['rate'] * (d.shape[1] // Q), MAX_CREDIT)
            while background and background[0][0] <= credit['left']:
                cost, work = background.popleft()
                credit['left'] -= cost
                work(d[r:r + 8, 0:Q])
        return d

    def dot(a, b):
        return release(jnp.dot(a, b, preferred_element_type=F32))

    def dot_nt(a, b):
        return release(lax.dot_general(a, b, (((1,), (1,)), ((), ())), preferred_element_type=F32))

    def token():
        return None if last[0] is None else last[0][0:8, 0:Q]

    def after(tok, x):
        if tok is None:
            return x
        if x.dtype == BF:
            return pltpu.bitcast(after(tok, pltpu.bitcast(x, I32)), BF)
        reps = (x.shape[0] // 8, x.shape[1] // Q)
        never = jnp.tile(inv_ref[0:8, :], reps) == 0
        return jnp.where(never, jnp.tile(pltpu.bitcast(tok, x.dtype), reps), x)

    def need(*what):
        while not done.issuperset(what):
            background.popleft()[1](token())

    lane = lax.broadcasted_iota(I32, (1, Q), 1)

    def operands(enc, terms, load, buf, height):
        def piece(r, o, tok):
            blk = {(i, j): {k: load(2 * i + k[0], 2 * j + k[1], r) for k in K2} for i, j in K2}
            blk[terms[o]] = {k: after(tok, v) for k, v in blk[terms[o]].items()}
            outer = {k: enc({q: blk[q][k].astype(F32) for q in K2})[o] for k in K2}
            for i, t in enumerate(enc(outer)):
                buf[7 * o + i, r:r + 16, :] = t.astype(BF)
        return [(50, P(piece, r, o)) for r in range(0, height, 16) for o in range(7)]

    def prepare_w3(j):
        cols = lambda h: slice(j * FC + h * Q, j * FC + (h + 1) * Q)

        def wide(tok):
            rest = [after(tok, w3b[4 * Q:D, cols(h)]).astype(F32) for h in range(4)]
            for i, t in enumerate(_wide2(_wide_b, rest)):
                w3r[j][i] = t.astype(BF)
            done.add(('w3', j))

        load = lambda k, h, r: w3b[k * Q + r:k * Q + r + 16, cols(h)]
        return operands(_enc_b, _TERM_B, load, w3a[j], Q) + [(150, wide)]

    def prepare_w4(j):
        load = lambda f, k, r: w4b[f * DQ + r:f * DQ + r + 16, j * FC + (3 - k) * Q:j * FC + (4 - k) * Q]
        return operands(_enc_a, _TERM_A, load, w4a[j], DQ) + [(0, lambda tok: done.add(('w4', j)))]

    def prepare_x(p, quarters):
        def wide(r, tok):
            for i, t in enumerate(_wide2(_wide_a, [x[r:r + 64, 4 * Q:] for x in quarters])):
                xr[p][i, r:r + 64, :] = t.astype(BF)

        load = lambda t, k, r: quarters[t][r:r + 16, k * Q:(k + 1) * Q]
        return (operands(_enc_a, _TERM_A, load, xa[p], Q) + [(150, P(wide, r)) for r in range(0, Q, 64)]
                + [(0, lambda tok: done.add(('x', p)))])

    conv = {'left': NG}

    def conv_load(u):
        rows = slice(16 * u, 16 * u + 16)
        prev = [jnp.zeros((16, Q), F32)] * KS
        for c in range(NC):
            cols = slice(c * Q, (c + 1) * Q)
            kc = kb[rows, cols].astype(F32)
            cur = [kc] + [pltpu.roll(kc, t, 1) for t in range(1, KS)]
            ks = kc * coef[0, rows, :]
            for t in range(1, KS):
                ks = ks + jnp.where(lane >= t, cur[t], prev[t]) * coef[t, rows, :]
            prev = cur
            taps = sb[rows, cols].astype(F32)
            if c == 0:
                taps = taps + jnp.where(lane == 0, coef[KS, rows, :], 0.0)
            conv['in', u, c] = (ks * vb[rows, cols].astype(F32), taps)

    def causal(a, b):
        out = [a[0] * x for x in b]
        for m in range(1, NC):
            for c in range(m, NC):
                out[c] = out[c] + a[m] * b[c - m]
        return out

    def conv_forward(g, part, tok):
        if part == 0 and g % 2 == 0:
            conv_load(g // 2)
        half = slice(8 * (g % 2), 8 * (g % 2) + 8)
        rows = jnp.concatenate([conv['in', g // 2, c][part == 0][half] for c in range(NC)], axis=0)
        lo, hi = ((0, 2), (0, 1), (1, 2))[part]
        t = dot(rows.astype(BF), pltpu.bitcast(fwd_ref[:, lo * Q:hi * Q], BF))
        conv.setdefault(g, []).extend([t[8 * c:8 * c + 8, n * Q:(n + 1) * Q] for c in range(NC)]
                                      for n in range(hi - lo))
        if part < 2:
            return
        kr, ki, ur, ui = conv.pop(g)
        e, f = [y - x for x, y in zip(ur, ui)], [x + y for x, y in zip(ur, ui)]
        a = [kr[0]] + [kr[m] - ki[m - 1] for m in range(1, NC)]
        b = [ki[0]] + [ki[m] + kr[m - 1] for m in range(1, NC)]
        s1, s2, s3 = causal([x + y for x, y in zip(a, b)], ur), causal(a, e), causal(b, f)
        conv['z', g] = (jnp.concatenate([x - y for x, y in zip(s1, s3)], axis=0),
                        jnp.concatenate([x + y for x, y in zip(s1, s2)], axis=0))

    def conv_inverse(g, tok):
        y = dot(jnp.concatenate(conv.pop(('z', g)), axis=1).astype(BF), pltpu.bitcast(inv_ref[...], BF))
        for c in range(NC):
            yb[8 * g:8 * g + 8, c * Q:(c + 1) * Q] = y[8 * c:8 * c + 8]
        conv['left'] -= 1

    def conv_step(g):
        for part, pause in enumerate(CONV_PAUSES):
            if g < NG:
                yield MATMUL + part, P(conv_forward, g, part)
            yield from [(100, lambda tok: None)] * pause
        if g >= 2:
            yield MATMUL + 3, P(conv_inverse, g - 2)

    mix = {}
    zero = jnp.zeros((DQ, Q), F32)

    def mix_dot(w, x):
        return jnp.concatenate([dot(w[:D // 2], x), dot(w[D // 2:], x)], axis=0)

    def mix_norm(b):
        cols = slice(b * TB, (b + 1) * TB)
        x = after(token(), xb[:, cols]).astype(F32)
        mix['x', b] = _layernorm(x).astype(BF)
        z = jnp.sum(x * jnp.tile(coef[KS + 1], (1, TB // Q)), axis=0, keepdims=True)
        gb[:, cols] = jnp.broadcast_to(1.0 / (1.0 + jnp.exp(-z)), (8, TB))

    def mix_first(b):
        h = _gelu(mix_dot(mix['w1'], mix.pop(('x', b))))
        for i in range(TB // Q):
            mix['h', b * (TB // Q) + i] = [pltpu.roll(h[g * DQ:(g + 1) * DQ, i * Q:(i + 1) * Q], shift, 1)
                                           for g, shift in enumerate((1, Q - 1, 2, Q - 2))]

    def shifted(c):
        lo = mix['h', c - 1] if c > 0 else [zero] * 4
        hi = mix['h', c + 1] if c + 1 < NC else [zero] * 4
        cur = mix['h', c]
        return jnp.concatenate([jnp.where(lane >= 1, cur[0], lo[0]),
                                jnp.where(lane < Q - 1, cur[1], hi[1]),
                                jnp.where(lane >= 2, cur[2], lo[2]),
                                jnp.where(lane < Q - 2, cur[3], hi[3])], axis=0)

    def mix_second(b):
        cols, n = slice(b * TB, (b + 1) * TB), TB // Q
        hs = jnp.concatenate([shifted(b * n + i) for i in range(n)], axis=1).astype(BF)
        x1 = xb[:, cols].astype(F32) + mix_dot(mix['w2'], hs) * UNSC
        x1b[:, cols] = x1
        y = _layernorm(x1)
        for i in range(n):
            mix['y', b * n + i] = y[:, i * Q:(i + 1) * Q].T
        if (b + 1) * TB % TP == 0:
            p = (b + 1) * TB // TP - 1
            background.extendleft(reversed(prepare_x(p, [mix.pop(('y', 4 * p + t)) for t in range(4)])))

    hidden = {}
    out = {}

    def up(p, j):
        m, h = {}, {}
        for stage, groups in enumerate(STAGE_GROUPS):
            parts = {}
            for item in STAGE_ORDER[len(groups)]:
                if item is None:
                    yield
                    continue
                o, i = groups[item[0]], item[1]
                parts[o, i] = dot(xa[p][7 * o + i], w3a[j][7 * o + i])
                if o in WIDE and i in WIDE:
                    n = 4 * WIDE.index(o) + WIDE.index(i)
                    parts[o, i] += dot(xr[p][n], w3r[j][n])
            for o in groups:
                m[o] = _dec([parts[o, i] for i in range(7)])
            (t, c), terms, fn = DECODE[stage]
            h[1 - c, t] = _blockwise(lambda *v: _gelu(fn(*v)), *(m[o] for o in terms))
            for o in (o for o in range(7) if DOWN_READY[o] == stage):
                blk = {k: _enc_b({q: h[q][k] if q in h else 0.0 for q in K2})[o] for k in K2}
                for i, v in enumerate(_enc_b({(k, n): blk[n, 1 - k] for k, n in K2})):
                    hidden[p, j, 7 * o + i] = v.astype(BF)

    def finish(p, f, t, a, b, mlp, tok):
        rows = slice((2 * f + a) * DQ, (2 * f + a + 1) * DQ)
        cols = slice(p * TP + (2 * t + b) * Q, p * TP + (2 * t + b + 1) * Q)
        val = x1b[rows, cols] if mlp is None else x1b[rows, cols] + mlp * UNSC
        if conv['left']:
            x1b[rows, cols] = val
            background.append((100, P(finish, p, f, t, a, b, None)))
        else:
            h3 = after(tok, xb[rows, cols]).astype(F32) * yb[rows, cols]
            ob[rows, cols] = (val + gb[0:1, cols] * (h3 - val)).astype(BF)

    def down(p, jg, o, i):
        n, js = 7 * o + i, range(jg * KD, (jg + 1) * KD)
        need(*(('w4', j) for j in js))
        d = None
        for j in js:
            e = dot_nt(w4a[j][n], hidden.pop((p, j, n)))
            d = e if d is None else d + e
        out[p, o, i] = out[p, o, i] + d if jg else d
        if jg < NJ // KD - 1 or i != DOWN_ORDER[-1]:
            return
        out[p, o] = _dec([out.pop((p, o, t)) for t in range(7)])
        for (f, t), terms, fn in DECODE:
            if o in terms and all((p, q) in out for q in terms):
                for (a, b), mlp in _blockwise(fn, *(out[p, q] for q in terms)).items():
                    finish(p, f, t, a, b, mlp, None)
                if conv['left']:
                    background.append((0, lambda tok, c=out_copy[p, f, t]: c.start()))
                else:
                    out_copy[p, f, t].start()

    start(*small_in, x_in[0], w1_in, x_in[1])
    wait(*small_in)
    taps = shift_ref[...].astype(F32)
    rows = [taps[t:t + 1] for t in range(KS)]
    rows += [r[...].astype(F32).reshape(1, D) for r in (ssmd_ref, gate_ref)]
    for i, r in enumerate(rows):
        coef[i] = jnp.broadcast_to(r, (Q, D)).T

    wait(x_in[0])
    mix_norm(0)
    mix_norm(1)
    wait(w1_in)
    start(x_in[2], w2_in, w3_in[0], w3_in[1], w4_in[0], w3_in[2], w4_in[1])
    mix['w1'] = w1b[...].astype(F32).T.astype(BF)
    mix_first(0)
    mix_first(1)
    wait(x_in[1])
    last[0] = None
    for kind, b in HEAD.split():
        if kind == 'x':
            wait(x_in[2], w2_in, w3_in[0])
            background.extend(prepare_w3(0) + prepare_w3(1))
            mix['w2'] = w2b[...].astype(F32).T.astype(BF)
        elif kind == 'w':
            wait(w3_in[1], w4_in[0])
            start(*conv_in)
            background.extend(prepare_w3(2) + [w for j in range(KD) for w in prepare_w4(j)])
        else:
            dict(n=mix_norm, f=mix_first, s=mix_second)[kind](int(b))
            continue
        last[0] = None
        credit['rate'] = RATES[kind]
    credit['rate'] = RATES['early']

    def last_inputs():
        wait(w3_in[2], w4_in[1], *conv_in)
        credit['rate'] = RATES['late']
        weights = lambda jg: [w for prepare in (prepare_w3, prepare_w4)
                              for j in range(jg * KD, (jg + 1) * KD) for w in prepare(j)]
        background.extend(weights(1))
        for g in range(NG + 2):
            if g == 16:
                background.extend(weights(2))
            background.extend(conv_step(g))

    def tick(n):
        if n == LAST_INPUTS_TICK:
            last_inputs()
        while background and background[0][0] >= MATMUL:
            if n is not None and n % 8 not in MATMUL_TICKS[background[0][0] - MATMUL]:
                break
            background.popleft()[1](None)

    blocks = [(jg, p) for jg in range(NJ // KD) for p in range(NP)]
    downs = collections.deque((4 * KD * (b + 1) - 3 + DOWN_READY[o], P(down, p, jg, o, i))
                              for b, (jg, p) in enumerate(blocks) for o in DOWN_ORDER for i in DOWN_ORDER)
    first, issued = downs[0][0] + DOWN_LAG, 0
    for b, (jg, p) in enumerate(blocks):
        for jj in range(KD):
            for n, _ in enumerate(up(p, jg * KD + jj)):
                stage, k = 4 * (KD * b + jj) + n // 4, n % 4
                tick(8 * stage + 2 * k)
                goal = (4 * (stage - first) + k + 1) * 49 // (16 * KD)
                while downs and issued < goal and downs[0][0] <= stage:
                    downs.popleft()[1]()
                    issued += 1
                tick(8 * stage + 2 * k + 1)
    for _, work in downs:
        work()
        tick(None)
    while background:
        background.popleft()[1](token())
    wait(*out_copy.values())


@jax.jit
def pallas_gated_mix__ssm_conv_h3__mixer_s_mlp__prompt_kernel(
    A_q: jax.Array,
    A_k: jax.Array,
    A_v: jax.Array,
    A_shift_k: jax.Array,
    A_ssm_k: jax.Array,
    A_ssm_D: jax.Array,
    B_x: jax.Array,
    B_w1: jax.Array,
    B_w2: jax.Array,
    B_w3: jax.Array,
    B_w4: jax.Array,
    gate_w: jax.Array,
):
    del B_x
    by_feature = lambda a: a.reshape(S, D).T
    hbm = pl.BlockSpec(memory_space=pl.ANY)
    scratch = (
        [pltpu.VMEM((KS, D), BF), pltpu.VMEM((D,), BF), pltpu.VMEM((D,), BF),
         pltpu.VMEM(_FWD.shape, I32), pltpu.VMEM(_INV.shape, I32)]
        + [pltpu.VMEM((D, S), BF)] * 4
        + [pltpu.VMEM((D, D), BF)] * 2
        + [pltpu.VMEM((D, F), BF)] * 2
        + [[pltpu.VMEM((49, Q, Q), BF)] * NP,
           [pltpu.VMEM((16, Q, DR), BF)] * NP,
           [pltpu.VMEM((49, Q, Q), BF)] * NJ,
           [pltpu.VMEM((16, DR, Q), BF)] * NJ,
           [pltpu.VMEM((49, DQ, Q), BF)] * NJ]
        + [pltpu.VMEM((KS + 2, D, Q), F32),
           pltpu.VMEM((D, S), F32),
           pltpu.VMEM((D, S), F32),
           pltpu.VMEM((8, S), F32),
           pltpu.VMEM((D, S), BF),
           pltpu.SemaphoreType.DMA((N_SEMS,))]
    )
    out = pl.pallas_call(
        _kernel,
        in_specs=[hbm] * 13,
        out_specs=hbm,
        out_shape=jax.ShapeDtypeStruct((D, S), BF),
        scratch_shapes=scratch,
        compiler_params=pltpu.CompilerParams(
            vmem_limit_bytes=126 * 1024 * 1024,
            flags={'XLA_TPU_EVENLY_DISTRIBUTE_CRITICAL_NODES': True}),
    )(A_shift_k.T, A_ssm_D, gate_w, jnp.asarray(_FWD), jnp.asarray(_INV),
      by_feature(A_q), by_feature(A_k), by_feature(A_v), A_ssm_k, B_w1, B_w2, B_w3, B_w4.T)
    return out.T.reshape(1, S, D)
```

```python
import collections
import functools

import numpy as np
import jax
import jax.numpy as jnp
from jax import lax
import jax.experimental.pallas as pl
import jax.experimental.pallas.tpu as pltpu

BF = jnp.bfloat16
F32 = jnp.float32
I32 = jnp.int32

S, D, F = 2048, 576, 4608
KS = 4
Q = 128
NC = S // Q
TP = 4 * Q
NP = S // TP
FC = 4 * Q
NJ = F // FC
KD = 3
DQ = D // 4
DR = D - 4 * Q
TB = 2 * Q
NG = D // 8
EPS = 1e-5
N_SEMS = 34

_C0 = float(np.sqrt(2.0 / np.pi))
SC = float((_C0 * 0.044715) ** (1.0 / 3.0))
AA = _C0 / SC
UNSC = 0.5 / SC


def _bf16_words(a):
    u = a.astype(np.float32).view(np.uint32)
    u = (u + 0x7FFF + ((u >> 16) & 1)) >> 16
    return (u[0::2] | (u[1::2] << 16)).astype(np.uint32).view(np.int32)


def _transform_matrices():
    theta = 2.0 * np.pi * (np.arange(Q) + 0.25) / Q
    ang = np.arange(Q)[:, None] * theta[None, :]
    fwd = np.concatenate([np.cos(ang), -np.sin(ang)], axis=1)
    inv = np.concatenate([np.cos(ang).T, -np.sin(ang).T], axis=0) / Q
    return _bf16_words(fwd), _bf16_words(inv)


_FWD, _INV = _transform_matrices()
assert (_INV[0:8] != 0).all()


def _gelu(xs):
    return xs * jnp.tanh(xs * (xs * xs + AA)) + xs


def _layernorm(x):
    mean = jnp.sum(x, axis=0, keepdims=True) * (1.0 / D)
    xc = x - mean
    var = jnp.sum(xc * xc, axis=0, keepdims=True) * (1.0 / D)
    scale = lax.rsqrt(var + EPS) * SC
    return x * scale - mean * scale


K2 = ((0, 0), (0, 1), (1, 0), (1, 1))
WIDE = (0, 3, 4, 6)


def _enc_a(a):
    return [a[0, 0] + a[1, 1], a[1, 0] + a[1, 1], a[0, 0], a[1, 1],
            a[0, 0] + a[0, 1], a[1, 0] - a[0, 0], a[0, 1] - a[1, 1]]


def _enc_b(b):
    return [b[0, 0] + b[1, 1], b[0, 0], b[0, 1] - b[1, 1], b[1, 0] - b[0, 0],
            b[1, 1], b[0, 0] + b[0, 1], b[1, 0] + b[1, 1]]


_TERM_A = ((0, 0), (1, 0), (0, 0), (1, 1), (0, 0), (1, 0), (0, 1))
_TERM_B = ((0, 0), (0, 0), (0, 1), (1, 0), (1, 1), (0, 0), (1, 0))


def _wide_a(a0, a1):
    return [a1, a1, a0, a0 - a1]


def _wide_b(b0, b1):
    return [b1, b0, b1, b0 + b1]


def _wide2(enc, quarters):
    outer = [enc(quarters[k], quarters[2 + k]) for k in range(2)]
    return [t for o in range(4) for t in enc(outer[0][o], outer[1][o])]


def _two(a, b):
    return a + b


def _four(a, b, c, d):
    return (a - b) + c + d


DECODE = (((0, 1), (2, 4), _two), ((1, 0), (1, 3), _two),
          ((0, 0), (3, 4, 0, 6), _four), ((1, 1), (2, 1, 0, 5), _four))


def _dec(m):
    return {blk: fn(*(m[i] for i in terms)) for blk, terms, fn in DECODE}


def _blockwise(fn, *ds):
    return {k: fn(*(d[k] for d in ds)) for k in K2}


STAGE_GROUPS = ((2, 4), (1, 3), (0, 6), (5,))
STAGE_ORDER = {
    1: ((0, 2), (0, 1), (0, 4), (0, 3), (0, 0), None, (0, 6), None, (0, 5), None, None),
    2: ((0, 1), (0, 2), (0, 4), None, (0, 3), (1, 3), (1, 2), (1, 4), (1, 1), None,
        (0, 0), (0, 5), (0, 6), None, (1, 0), (1, 6), None, (1, 5)),
}
DOWN_ORDER = (1, 4, 0, 3, 6, 2, 5)
DOWN_READY = {1: 0, 0: 1, 4: 1, 3: 2, 6: 2, 2: 3, 5: 3}
DOWN_LAG = 4
HEAD = 'n2 n3 f2 n4 f3 f4 x0 s0 n5 n6 n7 s1 s2 f5 f6 f7 w0 s3 s4 s5 s6 s7'
MATMUL = 1000
MATMUL_TICKS = ((2, 6), (0, 4), (0, 4), (2, 6))
CONV_PAUSES = (1, 2, 2)
LAST_INPUTS_TICK = 183
RATES = dict(x=1.4, w=2.3, early=0.33, late=0.195)
MAX_CREDIT = 200


def _kernel(shift_hbm, ssmd_hbm, gate_hbm, fwd_hbm, inv_hbm,
            x_hbm, k_hbm, v_hbm, s_hbm, w1_hbm, w2_hbm, w3_hbm, w4_hbm,
            o_hbm,
            shift_ref, ssmd_ref, gate_ref, fwd_ref, inv_ref,
            kb, vb, sb, xb, w1b, w2b, w3b, w4b, xa, xr, w3a, w3r, w4a, coef, x1b, yb, gb, ob,
            sem):
    P = functools.partial

    sems = iter(range(N_SEMS))

    def copy(src, dst, rows=(0, D), cols=None):
        if cols is not None:
            at = (pl.ds(rows[0], rows[1] - rows[0]), pl.ds(cols[0], cols[1] - cols[0]))
            src, dst = src.at[at], dst.at[at]
        return pltpu.make_async_copy(src, dst, sem.at[next(sems)])

    def start(*copies):
        for c in copies:
            c.start()

    def wait(*copies):
        for c in copies:
            c.wait()

    small_in = [copy(shift_hbm, shift_ref), copy(ssmd_hbm, ssmd_ref), copy(gate_hbm, gate_ref)]
    inv_in = copy(inv_hbm, inv_ref)
    x_in = [copy(x_hbm, xb, cols=c) for c in ((0, 2 * TB), (2 * TB, 5 * TB), (5 * TB, S))]
    w1_in, w2_in = copy(w1_hbm, w1b), copy(w2_hbm, w2b)
    w3_in = [copy(w3_hbm, w3b, cols=c) for c in ((0, 2 * FC), (2 * FC, KD * FC), (KD * FC, F))]
    w4_in = [copy(w4_hbm, w4b, cols=c) for c in ((0, KD * FC), (KD * FC, F))]
    conv_in = [copy(fwd_hbm, fwd_ref), copy(k_hbm, kb), copy(v_hbm, vb), copy(s_hbm, sb)]
    out_copy = {(p, f, t): copy(ob, o_hbm, (f * 2 * DQ, (f + 1) * 2 * DQ),
                                (p * TP + t * 2 * Q, p * TP + (t + 1) * 2 * Q))
                for p in range(NP) for f, t in K2}

    last = [None]
    done = set()
    background = collections.deque()
    credit = dict(left=0.0, rate=0.0)

    def release(d):
        last[0] = d
        for r in range(0, d.shape[0], 32):
            credit['left'] = min(credit['left'] + 32 * credit['rate'] * (d.shape[1] // Q), MAX_CREDIT)
            while background and background[0][0] <= credit['left']:
                cost, work = background.popleft()
                credit['left'] -= cost
                work(d[r:r + 8, 0:Q])
        return d

    def dot(a, b):
        return release(jnp.dot(a, b, preferred_element_type=F32))

    def dot_nt(a, b):
        return release(lax.dot_general(a, b, (((1,), (1,)), ((), ())), preferred_element_type=F32))

    def token():
        return None if last[0] is None else last[0][0:8, 0:Q]

    def after(tok, x):
        if tok is None:
            return x
        if x.dtype == BF:
            return pltpu.bitcast(after(tok, pltpu.bitcast(x, I32)), BF)
        reps = (x.shape[0] // 8, x.shape[1] // Q)
        never = jnp.tile(inv_ref[0:8, :], reps) == 0
        return jnp.where(never, jnp.tile(pltpu.bitcast(tok, x.dtype), reps), x)

    def need(*what):
        while not done.issuperset(what):
            background.popleft()[1](token())

    lane = lax.broadcasted_iota(I32, (1, Q), 1)

    def operands(enc, terms, load, buf, height):
        def piece(r, o, tok):
            blk = {(i, j): {k: load(2 * i + k[0], 2 * j + k[1], r) for k in K2} for i, j in K2}
            blk[terms[o]] = {k: after(tok, v) for k, v in blk[terms[o]].items()}
            outer = {k: enc({q: blk[q][k].astype(F32) for q in K2})[o] for k in K2}
            for i, t in enumerate(enc(outer)):
                buf[7 * o + i, r:r + 16, :] = t.astype(BF)
        return [(50, P(piece, r, o)) for r in range(0, height, 16) for o in range(7)]

    def prepare_w3(j):
        cols = lambda h: slice(j * FC + h * Q, j * FC + (h + 1) * Q)

        def wide(tok):
            rest = [after(tok, w3b[4 * Q:D, cols(h)]).astype(F32) for h in range(4)]
            for i, t in enumerate(_wide2(_wide_b, rest)):
                w3r[j][i] = t.astype(BF)
            done.add(('w3', j))

        load = lambda k, h, r: w3b[k * Q + r:k * Q + r + 16, cols(h)]
        return operands(_enc_b, _TERM_B, load, w3a[j], Q) + [(150, wide)]

    def prepare_w4(j):
        load = lambda f, k, r: w4b[f * DQ + r:f * DQ + r + 16, j * FC + (3 - k) * Q:j * FC + (4 - k) * Q]
        return operands(_enc_a, _TERM_A, load, w4a[j], DQ) + [(0, lambda tok: done.add(('w4', j)))]

    def prepare_x(p, quarters):
        def wide(r, tok):
            for i, t in enumerate(_wide2(_wide_a, [x[r:r + 64, 4 * Q:] for x in quarters])):
                xr[p][i, r:r + 64, :] = t.astype(BF)

        load = lambda t, k, r: quarters[t][r:r + 16, k * Q:(k + 1) * Q]
        return (operands(_enc_a, _TERM_A, load, xa[p], Q) + [(150, P(wide, r)) for r in range(0, Q, 64)]
                + [(0, lambda tok: done.add(('x', p)))])

    conv = {'left': NG}

    def conv_load(u):
        rows = slice(16 * u, 16 * u + 16)
        prev = [jnp.zeros((16, Q), F32)] * KS
        for c in range(NC):
            cols = slice(c * Q, (c + 1) * Q)
            kc = kb[rows, cols].astype(F32)
            cur = [kc] + [pltpu.roll(kc, t, 1) for t in range(1, KS)]
            ks = kc * coef[0, rows, :]
            for t in range(1, KS):
                ks = ks + jnp.where(lane >= t, cur[t], prev[t]) * coef[t, rows, :]
            prev = cur
            taps = sb[rows, cols].astype(F32)
            if c == 0:
                taps = taps + jnp.where(lane == 0, coef[KS, rows, :], 0.0)
            conv['in', u, c] = (ks * vb[rows, cols].astype(F32), taps)

    def causal(a, b):
        out = [a[0] * x for x in b]
        for m in range(1, NC):
            for c in range(m, NC):
                out[c] = out[c] + a[m] * b[c - m]
        return out

    def conv_forward(g, part, tok):
        if part == 0 and g % 2 == 0:
            conv_load(g // 2)
        half = slice(8 * (g % 2), 8 * (g % 2) + 8)
        rows = jnp.concatenate([conv['in', g // 2, c][part == 0][half] for c in range(NC)], axis=0)
        lo, hi = ((0, 2), (0, 1), (1, 2))[part]
        t = dot(rows.astype(BF), pltpu.bitcast(fwd_ref[:, lo * Q:hi * Q], BF))
        conv.setdefault(g, []).extend([t[8 * c:8 * c + 8, n * Q:(n + 1) * Q] for c in range(NC)]
                                      for n in range(hi - lo))
        if part < 2:
            return
        kr, ki, ur, ui = conv.pop(g)
        e, f = [y - x for x, y in zip(ur, ui)], [x + y for x, y in zip(ur, ui)]
        a = [kr[0]] + [kr[m] - ki[m - 1] for m in range(1, NC)]
        b = [ki[0]] + [ki[m] + kr[m - 1] for m in range(1, NC)]
        s1, s2, s3 = causal([x + y for x, y in zip(a, b)], ur), causal(a, e), causal(b, f)
        conv['z', g] = (jnp.concatenate([x - y for x, y in zip(s1, s3)], axis=0),
                        jnp.concatenate([x + y for x, y in zip(s1, s2)], axis=0))

    def conv_inverse(g, tok):
        y = dot(jnp.concatenate(conv.pop(('z', g)), axis=1).astype(BF), pltpu.bitcast(inv_ref[...], BF))
        for c in range(NC):
            yb[8 * g:8 * g + 8, c * Q:(c + 1) * Q] = y[8 * c:8 * c + 8]
        conv['left'] -= 1

    def conv_step(g):
        for part, pause in enumerate(CONV_PAUSES):
            if g < NG:
                yield MATMUL + part, P(conv_forward, g, part)
            yield from [(100, lambda tok: None)] * pause
        if g >= 2:
            yield MATMUL + 3, P(conv_inverse, g - 2)

    mix = {}
    zero = jnp.zeros((DQ, Q), F32)

    def mix_dot(w, x):
        return jnp.concatenate([dot(w[:D // 2], x), dot(w[D // 2:], x)], axis=0)

    def mix_norm(b):
        cols = slice(b * TB, (b + 1) * TB)
        x = after(token(), xb[:, cols]).astype(F32)
        mix['x', b] = _layernorm(x).astype(BF)
        z = jnp.sum(x * jnp.tile(coef[KS + 1], (1, TB // Q)), axis=0, keepdims=True)
        gb[:, cols] = jnp.broadcast_to(1.0 / (1.0 + jnp.exp(-z)), (8, TB))

    def mix_first(b):
        h = _gelu(mix_dot(mix['w1'], mix.pop(('x', b))))
        for i in range(TB // Q):
            mix['h', b * (TB // Q) + i] = [pltpu.roll(h[g * DQ:(g + 1) * DQ, i * Q:(i + 1) * Q], shift, 1)
                                           for g, shift in enumerate((1, Q - 1, 2, Q - 2))]

    def shifted(c):
        lo = mix['h', c - 1] if c > 0 else [zero] * 4
        hi = mix['h', c + 1] if c + 1 < NC else [zero] * 4
        cur = mix['h', c]
        return jnp.concatenate([jnp.where(lane >= 1, cur[0], lo[0]),
                                jnp.where(lane < Q - 1, cur[1], hi[1]),
                                jnp.where(lane >= 2, cur[2], lo[2]),
                                jnp.where(lane < Q - 2, cur[3], hi[3])], axis=0)

    def mix_second(b):
        cols, n = slice(b * TB, (b + 1) * TB), TB // Q
        hs = jnp.concatenate([shifted(b * n + i) for i in range(n)], axis=1).astype(BF)
        x1 = xb[:, cols].astype(F32) + mix_dot(mix['w2'], hs) * UNSC
        x1b[:, cols] = x1
        y = _layernorm(x1)
        for i in range(n):
            mix['y', b * n + i] = y[:, i * Q:(i + 1) * Q].T
        if (b + 1) * TB % TP == 0:
            p = (b + 1) * TB // TP - 1
            background.extendleft(reversed(prepare_x(p, [mix.pop(('y', 4 * p + t)) for t in range(4)])))

    hidden = {}
    out = {}

    def up(p, j):
        m, h = {}, {}
        for stage, groups in enumerate(STAGE_GROUPS):
            parts = {}
            for item in STAGE_ORDER[len(groups)]:
                if item is None:
                    yield
                    continue
                o, i = groups[item[0]], item[1]
                if o in WIDE and i in WIDE:
                    n = 4 * WIDE.index(o) + WIDE.index(i)
                    rest = dot(xr[p][n], w3r[j][n])
                    parts[o, i] = rest + dot(xa[p][7 * o + i], w3a[j][7 * o + i])
                else:
                    parts[o, i] = dot(xa[p][7 * o + i], w3a[j][7 * o + i])
            for o in groups:
                m[o] = _dec([parts[o, i] for i in range(7)])
            (t, c), terms, fn = DECODE[stage]
            h[1 - c, t] = _blockwise(lambda *v: _gelu(fn(*v)), *(m[o] for o in terms))
            for o in (o for o in range(7) if DOWN_READY[o] == stage):
                blk = {k: _enc_b({q: h[q][k] if q in h else 0.0 for q in K2})[o] for k in K2}
                for i, v in enumerate(_enc_b({(k, n): blk[n, 1 - k] for k, n in K2})):
                    hidden[p, j, 7 * o + i] = v.astype(BF)

    def finish(p, f, t, a, b, mlp, tok):
        rows = slice((2 * f + a) * DQ, (2 * f + a + 1) * DQ)
        cols = slice(p * TP + (2 * t + b) * Q, p * TP + (2 * t + b + 1) * Q)
        val = x1b[rows, cols] if mlp is None else x1b[rows, cols] + mlp * UNSC
        if conv['left']:
            x1b[rows, cols] = val
            background.append((100, P(finish, p, f, t, a, b, None)))
        else:
            h3 = after(tok, xb[rows, cols]).astype(F32) * yb[rows, cols]
            ob[rows, cols] = (val + gb[0:1, cols] * (h3 - val)).astype(BF)

    def down(p, jg, o, i):
        n, js = 7 * o + i, range(jg * KD, (jg + 1) * KD)
        need(*(('w4', j) for j in js))
        d = None
        for j in js:
            e = dot_nt(w4a[j][n], hidden.pop((p, j, n)))
            d = e if d is None else d + e
        out[p, o, i] = out[p, o, i] + d if jg else d
        if jg < NJ // KD - 1 or i != DOWN_ORDER[-1]:
            return
        out[p, o] = _dec([out.pop((p, o, t)) for t in range(7)])
        for (f, t), terms, fn in DECODE:
            if o in terms and all((p, q) in out for q in terms):
                for (a, b), mlp in _blockwise(fn, *(out[p, q] for q in terms)).items():
                    finish(p, f, t, a, b, mlp, None)
                if conv['left']:
                    background.append((0, lambda tok, c=out_copy[p, f, t]: c.start()))
                else:
                    out_copy[p, f, t].start()

    start(*small_in, x_in[0], w1_in, inv_in, x_in[1])
    wait(*small_in)
    taps = shift_ref[...].astype(F32)
    rows = [taps[t:t + 1] for t in range(KS)]
    rows += [r[...].astype(F32).reshape(1, D) for r in (ssmd_ref, gate_ref)]
    for i, r in enumerate(rows):
        coef[i] = jnp.broadcast_to(r, (Q, D)).T

    wait(x_in[0])
    mix_norm(0)
    mix_norm(1)
    wait(w1_in)
    start(x_in[2], w2_in, w3_in[0], w3_in[1], w4_in[0], w3_in[2], w4_in[1])
    mix['w1'] = w1b[...].astype(F32).T.astype(BF)
    mix_first(0)
    mix_first(1)
    wait(inv_in, x_in[1])
    last[0] = None
    for kind, b in HEAD.split():
        if kind == 'x':
            wait(x_in[2], w2_in, w3_in[0])
            background.extend(prepare_w3(0) + prepare_w3(1))
            mix['w2'] = w2b[...].astype(F32).T.astype(BF)
        elif kind == 'w':
            wait(w3_in[1], w4_in[0])
            start(*conv_in)
            background.extend(prepare_w3(2) + [w for j in range(KD) for w in prepare_w4(j)])
        else:
            dict(n=mix_norm, f=mix_first, s=mix_second)[kind](int(b))
            continue
        last[0] = None
        credit['rate'] = RATES[kind]
    credit['rate'] = RATES['early']

    def last_inputs():
        wait(w3_in[2], w4_in[1], *conv_in)
        credit['rate'] = RATES['late']
        weights = lambda jg: [w for prepare in (prepare_w3, prepare_w4)
                              for j in range(jg * KD, (jg + 1) * KD) for w in prepare(j)]
        background.extend(weights(1))
        for g in range(NG + 2):
            if g == NG // 3:
                background.extend(weights(2))
            background.extend(conv_step(g))

    def tick(n):
        if n == LAST_INPUTS_TICK:
            last_inputs()
        while background and background[0][0] >= MATMUL:
            if n is not None and n % 8 not in MATMUL_TICKS[background[0][0] - MATMUL]:
                break
            background.popleft()[1](None)

    blocks = [(jg, p) for jg in range(NJ // KD) for p in range(NP)]
    downs = collections.deque((4 * KD * (b + 1) - 3 + DOWN_READY[o], P(down, p, jg, o, i))
                              for b, (jg, p) in enumerate(blocks) for o in DOWN_ORDER for i in DOWN_ORDER)
    first, issued = downs[0][0] + DOWN_LAG, 0
    for b, (jg, p) in enumerate(blocks):
        for jj in range(KD):
            for n, _ in enumerate(up(p, jg * KD + jj)):
                stage, k = 4 * (KD * b + jj) + n // 4, n % 4
                tick(8 * stage + 2 * k)
                goal = (4 * (stage - first) + k + 1) * 49 // (16 * KD)
                while downs and issued < goal and downs[0][0] <= stage:
                    downs.popleft()[1]()
                    issued += 1
                tick(8 * stage + 2 * k + 1)
    for _, work in downs:
        work()
        tick(None)
    while background:
        background.popleft()[1](token())
    wait(*out_copy.values())


@jax.jit
def pallas_gated_mix__ssm_conv_h3__mixer_s_mlp__prompt_kernel(
    A_q: jax.Array,
    A_k: jax.Array,
    A_v: jax.Array,
    A_shift_k: jax.Array,
    A_ssm_k: jax.Array,
    A_ssm_D: jax.Array,
    B_x: jax.Array,
    B_w1: jax.Array,
    B_w2: jax.Array,
    B_w3: jax.Array,
    B_w4: jax.Array,
    gate_w: jax.Array,
):
    del B_x
    by_feature = lambda a: a.reshape(S, D).T
    hbm = pl.BlockSpec(memory_space=pl.ANY)
    scratch = (
        [pltpu.VMEM((KS, D), BF), pltpu.VMEM((D,), BF), pltpu.VMEM((D,), BF),
         pltpu.VMEM(_FWD.shape, I32), pltpu.VMEM(_INV.shape, I32)]
        + [pltpu.VMEM((D, S), BF)] * 4
        + [pltpu.VMEM((D, D), BF)] * 2
        + [pltpu.VMEM((D, F), BF)] * 2
        + [[pltpu.VMEM((49, Q, Q), BF)] * NP,
           [pltpu.VMEM((16, Q, DR), BF)] * NP,
           [pltpu.VMEM((49, Q, Q), BF)] * NJ,
           [pltpu.VMEM((16, DR, Q), BF)] * NJ,
           [pltpu.VMEM((49, DQ, Q), BF)] * NJ]
        + [pltpu.VMEM((KS + 2, D, Q), F32),
           pltpu.VMEM((D, S), F32),
           pltpu.VMEM((D, S), F32),
           pltpu.VMEM((8, S), F32),
           pltpu.VMEM((D, S), BF),
           pltpu.SemaphoreType.DMA((N_SEMS,))]
    )
    out = pl.pallas_call(
        _kernel,
        in_specs=[hbm] * 13,
        out_specs=hbm,
        out_shape=jax.ShapeDtypeStruct((D, S), BF),
        scratch_shapes=scratch,
        compiler_params=pltpu.CompilerParams(
            vmem_limit_bytes=126 * 1024 * 1024,
            flags={'XLA_TPU_EVENLY_DISTRIBUTE_CRITICAL_NODES': True}),
    )(A_shift_k.T, A_ssm_D, gate_w, jnp.asarray(_FWD), jnp.asarray(_INV),
      by_feature(A_q), by_feature(A_k), by_feature(A_v), A_ssm_k, B_w1, B_w2, B_w3, B_w4.T)
    return out.T.reshape(1, S, D)
```

```python
import collections
import functools

import numpy as np
import jax
import jax.numpy as jnp
from jax import lax
import jax.experimental.pallas as pl
import jax.experimental.pallas.tpu as pltpu

BF = jnp.bfloat16
F32 = jnp.float32
I32 = jnp.int32

S, D, F = 2048, 576, 4608
KS = 4
Q = 128
NC = S // Q
TP = 4 * Q
NP = S // TP
FC = 4 * Q
NJ = F // FC
KD = 3
DQ = D // 4
DR = D - 4 * Q
TB = 2 * Q
NG = D // 8
EPS = 1e-5

_C0 = float(np.sqrt(2.0 / np.pi))
SC = float((_C0 * 0.044715) ** (1.0 / 3.0))
AA = _C0 / SC
UNSC = 0.5 / SC


def _bf16_words(a):
    u = a.astype(np.float32).view(np.uint32)
    u = (u + 0x7FFF + ((u >> 16) & 1)) >> 16
    return (u[0::2] | (u[1::2] << 16)).astype(np.uint32).view(np.int32)


def _transform_matrices():
    theta = 2.0 * np.pi * (np.arange(Q) + 0.25) / Q
    ang = np.arange(Q)[:, None] * theta[None, :]
    fwd = np.concatenate([np.cos(ang), -np.sin(ang)], axis=1)
    inv = np.concatenate([np.cos(ang).T, -np.sin(ang).T], axis=0) / Q
    return _bf16_words(fwd), _bf16_words(inv)


_FWD, _INV = _transform_matrices()
assert (_INV[0:8] != 0).all()


def _gelu(xs):
    return xs * (jnp.tanh(xs * (xs * xs + AA)) + 1.0)


def _layernorm(x):
    mean = jnp.sum(x, axis=0, keepdims=True) * (1.0 / D)
    xc = x - mean
    var = jnp.sum(xc * xc, axis=0, keepdims=True) * (1.0 / D)
    scale = lax.rsqrt(var + EPS) * SC
    return x * scale - mean * scale


K2 = ((0, 0), (0, 1), (1, 0), (1, 1))
WIDE = (0, 3, 4, 6)


def _enc_a(a):
    return [a[0, 0] + a[1, 1], a[1, 0] + a[1, 1], a[0, 0], a[1, 1],
            a[0, 0] + a[0, 1], a[1, 0] - a[0, 0], a[0, 1] - a[1, 1]]


def _enc_b(b):
    return [b[0, 0] + b[1, 1], b[0, 0], b[0, 1] - b[1, 1], b[1, 0] - b[0, 0],
            b[1, 1], b[0, 0] + b[0, 1], b[1, 0] + b[1, 1]]


_TERM_A = ((0, 0), (1, 0), (0, 0), (1, 1), (0, 0), (1, 0), (0, 1))
_TERM_B = ((0, 0), (0, 0), (0, 1), (1, 0), (1, 1), (0, 0), (1, 0))


def _wide_a(a0, a1):
    return [a1, a1, a0, a0 - a1]


def _wide_b(b0, b1):
    return [b1, b0, b1, b0 + b1]


def _wide2(enc, quarters):
    outer = [enc(quarters[k], quarters[2 + k]) for k in range(2)]
    return [t for o in range(4) for t in enc(outer[0][o], outer[1][o])]


def _two(a, b):
    return a + b


def _four(a, b, c, d):
    return (a - b) + c + d


DECODE = (((0, 1), (2, 4), _two), ((1, 0), (1, 3), _two),
          ((0, 0), (3, 4, 0, 6), _four), ((1, 1), (2, 1, 0, 5), _four))


def _dec(m):
    return {blk: fn(*(m[i] for i in terms)) for blk, terms, fn in DECODE}


def _blockwise(fn, *ds):
    return {k: fn(*(d[k] for d in ds)) for k in K2}


STAGE_GROUPS = ((2, 4), (1, 3), (0, 6), (5,))
STAGE_ORDER = {
    1: ((0, 2), (0, 1), (0, 4), (0, 3), (0, 0), None, (0, 6), None, None, None, (0, 5)),
    2: ((0, 1), (0, 2), (0, 4), None, (0, 3), (1, 3), (1, 2), (1, 4), (1, 1), None,
        (0, 0), (0, 5), (0, 6), None, (1, 0), (1, 6), None, (1, 5)),
}
DOWN_ORDER = (1, 4, 0, 3, 6, 2, 5)
DOWN_READY = {1: 0, 0: 1, 4: 1, 3: 2, 6: 2, 2: 3, 5: 3}
DOWN_LAG = 4
HEAD = 'n2 n3 f2 n4 f3 n5 f4 f5 x0 s0 n6 s1 n7 s2 f6 f7 w0 s3 s4 s5 s6 s7'
MATMUL = 1000
MATMUL_TICKS = ((2, 6), (0, 4), (0, 4), (2, 6))
CONV_PAUSES = (1, 2, 2)
LAST_INPUTS_TICK = 183
RATES = dict(x=1.4, w=2.3, early=0.33, late=0.2)
MAX_CREDIT = 200


def _kernel(shift_hbm, ssmd_hbm, gate_hbm, fwd_hbm, inv_hbm,
            x_hbm, k_hbm, v_hbm, s_hbm, w1_hbm, w2_hbm, w3_hbm, w4_hbm,
            o_hbm,
            shift_ref, ssmd_ref, gate_ref, fwd_ref, inv_ref,
            kb, vb, sb, xb, w1b, w2b, w3b, w4b, xa, xr, w3a, w3r, w4a, coef, x1b, yb, gb, ob,
            sem):
    P = functools.partial

    def group(n, *parts):
        copies = []
        for src, dst, *window in parts:
            if window:
                at = tuple(pl.ds(lo, hi - lo) for lo, hi in window)
                src, dst = src.at[at], dst.at[at]
            copies.append(pltpu.make_async_copy(src, dst, sem.at[n]))
        return copies

    def start(copies):
        for c in copies:
            c.start()

    def wait(copies):
        for c in copies:
            c.wait()

    columns = lambda src, dst, lo, hi: (src, dst, (0, D), (lo, hi))
    inputs = [
        group(0, (shift_hbm, shift_ref), (ssmd_hbm, ssmd_ref), (gate_hbm, gate_ref)),
        group(1, columns(x_hbm, xb, 0, TB)),
        group(2, (w1_hbm, w1b), columns(x_hbm, xb, TB, 2 * TB)),
        group(3, (inv_hbm, inv_ref), columns(x_hbm, xb, 2 * TB, 6 * TB)),
        group(4, columns(x_hbm, xb, 6 * TB, S), (w2_hbm, w2b), columns(w3_hbm, w3b, 0, 2 * FC)),
        group(5, columns(w3_hbm, w3b, 2 * FC, KD * FC), columns(w4_hbm, w4b, 0, KD * FC)),
        group(6, columns(w3_hbm, w3b, KD * FC, F), columns(w4_hbm, w4b, KD * FC, F),
              (fwd_hbm, fwd_ref), (k_hbm, kb), (v_hbm, vb), (s_hbm, sb)),
    ]
    out_blocks = [(p, f, t) for p in range(NP) for f, t in K2]
    out_copy = dict(zip(out_blocks, group(7, *(
        (ob, o_hbm, (f * 2 * DQ, (f + 1) * 2 * DQ), (p * TP + t * 2 * Q, p * TP + (t + 1) * 2 * Q))
        for p, f, t in out_blocks))))

    last = [None]
    done = set()
    background = collections.deque()
    credit = dict(left=0.0, rate=0.0)

    def release(d):
        last[0] = d
        for r in range(0, d.shape[0], 32):
            credit['left'] = min(credit['left'] + 32 * credit['rate'] * (d.shape[1] // Q), MAX_CREDIT)
            while background and background[0][0] <= credit['left']:
                cost, work = background.popleft()
                credit['left'] -= cost
                work(d[r:r + 8, 0:Q])
        return d

    def dot(a, b):
        return release(jnp.dot(a, b, preferred_element_type=F32))

    def dot_nt(a, b):
        return release(lax.dot_general(a, b, (((1,), (1,)), ((), ())), preferred_element_type=F32))

    def token():
        return None if last[0] is None else last[0][0:8, 0:Q]

    def after(tok, x):
        if tok is None:
            return x
        if x.dtype == BF:
            return pltpu.bitcast(after(tok, pltpu.bitcast(x, I32)), BF)
        reps = (x.shape[0] // 8, x.shape[1] // Q)
        never = jnp.tile(inv_ref[0:8, :], reps) == 0
        return jnp.where(never, jnp.tile(pltpu.bitcast(tok, x.dtype), reps), x)

    def need(*what):
        while not done.issuperset(what):
            background.popleft()[1](token())

    lane = lax.broadcasted_iota(I32, (1, Q), 1)

    def operands(enc, terms, load, buf, height):
        def piece(r, o, tok):
            blk = {(i, j): {k: load(2 * i + k[0], 2 * j + k[1], r) for k in K2} for i, j in K2}
            blk[terms[o]] = {k: after(tok, v) for k, v in blk[terms[o]].items()}
            outer = {k: enc({q: blk[q][k].astype(F32) for q in K2})[o] for k in K2}
            for i, t in enumerate(enc(outer)):
                buf[7 * o + i, r:r + 16, :] = t.astype(BF)
        return [(50, P(piece, r, o)) for r in range(0, height, 16) for o in range(7)]

    def prepare_w3(j):
        cols = lambda h: slice(j * FC + h * Q, j * FC + (h + 1) * Q)

        def wide(tok):
            rest = [after(tok, w3b[4 * Q:D, cols(h)]).astype(F32) for h in range(4)]
            for i, t in enumerate(_wide2(_wide_b, rest)):
                w3r[j][i] = t.astype(BF)
            done.add(('w3', j))

        load = lambda k, h, r: w3b[k * Q + r:k * Q + r + 16, cols(h)]
        return operands(_enc_b, _TERM_B, load, w3a[j], Q) + [(150, wide)]

    def prepare_w4(j):
        load = lambda f, k, r: w4b[f * DQ + r:f * DQ + r + 16, j * FC + (3 - k) * Q:j * FC + (4 - k) * Q]
        return operands(_enc_a, _TERM_A, load, w4a[j], DQ) + [(0, lambda tok: done.add(('w4', j)))]

    def prepare_x(p, quarters):
        def wide(r, tok):
            for i, t in enumerate(_wide2(_wide_a, [x[r:r + 64, 4 * Q:] for x in quarters])):
                xr[p][i, r:r + 64, :] = t.astype(BF)

        load = lambda t, k, r: quarters[t][r:r + 16, k * Q:(k + 1) * Q]
        return (operands(_enc_a, _TERM_A, load, xa[p], Q) + [(150, P(wide, r)) for r in range(0, Q, 64)]
                + [(0, lambda tok: done.add(('x', p)))])

    conv = {'left': NG}

    def conv_load(u):
        rows = slice(16 * u, 16 * u + 16)
        prev = [jnp.zeros((16, Q), F32)] * KS
        for c in range(NC):
            cols = slice(c * Q, (c + 1) * Q)
            kc = kb[rows, cols].astype(F32)
            cur = [kc] + [pltpu.roll(kc, t, 1) for t in range(1, KS)]
            ks = kc * coef[0, rows, :]
            for t in range(1, KS):
                ks = ks + jnp.where(lane >= t, cur[t], prev[t]) * coef[t, rows, :]
            prev = cur
            taps = sb[rows, cols].astype(F32)
            if c == 0:
                taps = taps + jnp.where(lane == 0, coef[KS, rows, :], 0.0)
            conv['in', u, c] = (ks * vb[rows, cols].astype(F32), taps)

    def causal(a, b):
        out = [a[0] * x for x in b]
        for m in range(1, NC):
            for c in range(m, NC):
                out[c] = out[c] + a[m] * b[c - m]
        return out

    def conv_forward(g, part, tok):
        if part == 0 and g % 2 == 0:
            conv_load(g // 2)
        half = slice(8 * (g % 2), 8 * (g % 2) + 8)
        rows = jnp.concatenate([conv['in', g // 2, c][part == 0][half] for c in range(NC)], axis=0)
        lo, hi = ((0, 2), (0, 1), (1, 2))[part]
        t = dot(rows.astype(BF), pltpu.bitcast(fwd_ref[:, lo * Q:hi * Q], BF))
        conv.setdefault(g, []).extend([t[8 * c:8 * c + 8, n * Q:(n + 1) * Q] for c in range(NC)]
                                      for n in range(hi - lo))
        if part < 2:
            return
        kr, ki, ur, ui = conv.pop(g)
        e, f = [y - x for x, y in zip(ur, ui)], [x + y for x, y in zip(ur, ui)]
        a = [kr[0]] + [kr[m] - ki[m - 1] for m in range(1, NC)]
        b = [ki[0]] + [ki[m] + kr[m - 1] for m in range(1, NC)]
        s1, s2, s3 = causal([x + y for x, y in zip(a, b)], ur), causal(a, e), causal(b, f)
        conv['z', g] = (jnp.concatenate([x - y for x, y in zip(s1, s3)], axis=0),
                        jnp.concatenate([x + y for x, y in zip(s1, s2)], axis=0))

    def conv_inverse(g, tok):
        y = dot(jnp.concatenate(conv.pop(('z', g)), axis=1).astype(BF), pltpu.bitcast(inv_ref[...], BF))
        for c in range(NC):
            yb[8 * g:8 * g + 8, c * Q:(c + 1) * Q] = y[8 * c:8 * c + 8]
        conv['left'] -= 1

    def conv_step(g):
        for part, pause in enumerate(CONV_PAUSES):
            if g < NG:
                yield MATMUL + part, P(conv_forward, g, part)
            yield from [(100, lambda tok: None)] * pause
        if g:
            yield MATMUL + 3, P(conv_inverse, g - 1)

    mix = {}
    zero = jnp.zeros((DQ, Q), F32)

    def mix_dot(w, x):
        return jnp.concatenate([dot(w[:D // 2], x), dot(w[D // 2:], x)], axis=0)

    def mix_norm(b):
        cols = slice(b * TB, (b + 1) * TB)
        x = after(token(), xb[:, cols]).astype(F32)
        mix['x', b] = _layernorm(x).astype(BF)
        z = jnp.sum(x * jnp.tile(coef[KS + 1], (1, TB // Q)), axis=0, keepdims=True)
        gb[:, cols] = jnp.broadcast_to(1.0 / (1.0 + jnp.exp(-z)), (8, TB))

    def mix_first(b):
        h = _gelu(mix_dot(mix['w1'], mix.pop(('x', b))))
        for i in range(TB // Q):
            mix['h', b * (TB // Q) + i] = [pltpu.roll(h[g * DQ:(g + 1) * DQ, i * Q:(i + 1) * Q], shift, 1)
                                           for g, shift in enumerate((1, Q - 1, 2, Q - 2))]

    def shifted(c):
        lo = mix['h', c - 1] if c > 0 else [zero] * 4
        hi = mix['h', c + 1] if c + 1 < NC else [zero] * 4
        cur = mix['h', c]
        return jnp.concatenate([jnp.where(lane >= 1, cur[0], lo[0]),
                                jnp.where(lane < Q - 1, cur[1], hi[1]),
                                jnp.where(lane >= 2, cur[2], lo[2]),
                                jnp.where(lane < Q - 2, cur[3], hi[3])], axis=0)

    def mix_second(b):
        cols, n = slice(b * TB, (b + 1) * TB), TB // Q
        hs = jnp.concatenate([shifted(b * n + i) for i in range(n)], axis=1).astype(BF)
        x1 = xb[:, cols].astype(F32) + mix_dot(mix['w2'], hs) * UNSC
        x1b[:, cols] = x1
        y = _layernorm(x1)
        for i in range(n):
            mix['y', b * n + i] = y[:, i * Q:(i + 1) * Q].T
        if (b + 1) * TB % TP == 0:
            p = (b + 1) * TB // TP - 1
            background.extendleft(reversed(prepare_x(p, [mix.pop(('y', 4 * p + t)) for t in range(4)])))

    hidden = {}
    out = {}

    def up(p, j):
        m, h = {}, {}
        for stage, groups in enumerate(STAGE_GROUPS):
            parts = {}
            for item in STAGE_ORDER[len(groups)]:
                if item is None:
                    yield
                    continue
                o, i = groups[item[0]], item[1]
                if o in WIDE and i in WIDE:
                    n = 4 * WIDE.index(o) + WIDE.index(i)
                    rest = dot(xr[p][n], w3r[j][n])
                    parts[o, i] = rest + dot(xa[p][7 * o + i], w3a[j][7 * o + i])
                else:
                    parts[o, i] = dot(xa[p][7 * o + i], w3a[j][7 * o + i])
            for o in groups:
                m[o] = _dec([parts[o, i] for i in range(7)])
            (t, c), terms, fn = DECODE[stage]
            h[1 - c, t] = _blockwise(lambda *v: _gelu(fn(*v)), *(m[o] for o in terms))
            for o in (o for o in range(7) if DOWN_READY[o] == stage):
                blk = {k: _enc_b({q: h[q][k] if q in h else 0.0 for q in K2})[o] for k in K2}
                for i, v in enumerate(_enc_b({(k, n): blk[n, 1 - k] for k, n in K2})):
                    hidden[p, j, 7 * o + i] = v.astype(BF)

    def finish(p, f, t, a, b, mlp, tok):
        rows = slice((2 * f + a) * DQ, (2 * f + a + 1) * DQ)
        cols = slice(p * TP + (2 * t + b) * Q, p * TP + (2 * t + b + 1) * Q)
        val = x1b[rows, cols] if mlp is None else x1b[rows, cols] + mlp * UNSC
        if conv['left']:
            x1b[rows, cols] = val
            background.append((100, P(finish, p, f, t, a, b, None)))
        else:
            h3 = after(tok, xb[rows, cols]).astype(F32) * yb[rows, cols]
            ob[rows, cols] = (val + gb[0:1, cols] * (h3 - val)).astype(BF)

    def down(p, jg, o, i):
        n, js = 7 * o + i, range(jg * KD, (jg + 1) * KD)
        need(*(('w4', j) for j in js))
        d0, d1, d2 = (dot_nt(w4a[j][n], hidden.pop((p, j, n))) for j in js)
        d = d0 + (d1 + d2)
        out[p, o, i] = out[p, o, i] + d if jg else d
        if jg < NJ // KD - 1 or i != DOWN_ORDER[-1]:
            return
        out[p, o] = _dec([out.pop((p, o, t)) for t in range(7)])
        for (f, t), terms, fn in DECODE:
            if o in terms and all((p, q) in out for q in terms):
                for (a, b), mlp in _blockwise(fn, *(out[p, q] for q in terms)).items():
                    finish(p, f, t, a, b, mlp, None)
                if conv['left']:
                    background.append((0, lambda tok, c=out_copy[p, f, t]: c.start()))
                else:
                    out_copy[p, f, t].start()

    start(inputs[0] + inputs[1] + inputs[2] + inputs[3])
    wait(inputs[0])
    taps = shift_ref[...].astype(F32)
    rows = [taps[t:t + 1] for t in range(KS)]
    rows += [r[...].astype(F32).reshape(1, D) for r in (ssmd_ref, gate_ref)]
    for i, r in enumerate(rows):
        coef[i] = jnp.broadcast_to(r, (Q, D)).T

    wait(inputs[1])
    mix_norm(0)
    wait(inputs[2])
    mix_norm(1)
    start(inputs[4] + inputs[5] + inputs[6])
    mix['w1'] = w1b[...].astype(F32).T.astype(BF)
    mix_first(0)
    mix_first(1)
    wait(inputs[3])
    last[0] = None
    for kind, b in HEAD.split():
        if kind == 'x':
            wait(inputs[4])
            background.extend(prepare_w3(0) + prepare_w3(1))
            mix['w2'] = w2b[...].astype(F32).T.astype(BF)
        elif kind == 'w':
            wait(inputs[5])
            background.extend(prepare_w3(2) + [w for j in range(KD) for w in prepare_w4(j)])
        else:
            dict(n=mix_norm, f=mix_first, s=mix_second)[kind](int(b))
            continue
        last[0] = None
        credit['rate'] = RATES[kind]
    credit['rate'] = RATES['early']

    def last_inputs():
        wait(inputs[6])
        credit['rate'] = RATES['late']
        weights = lambda jg: [w for prepare in (prepare_w3, prepare_w4)
                              for j in range(jg * KD, (jg + 1) * KD) for w in prepare(j)]
        background.extend(weights(1))
        for g in range(NG + 1):
            if g == NG // 3:
                background.extend(weights(2))
            background.extend(conv_step(g))

    def tick(n):
        if n == LAST_INPUTS_TICK:
            last_inputs()
        while background and background[0][0] >= MATMUL:
            if n is not None and n % 8 not in MATMUL_TICKS[background[0][0] - MATMUL]:
                break
            background.popleft()[1](None)

    blocks = [(jg, p) for jg in range(NJ // KD) for p in range(NP)]
    downs = collections.deque((4 * KD * (b + 1) - 3 + DOWN_READY[o], P(down, p, jg, o, i))
                              for b, (jg, p) in enumerate(blocks) for o in DOWN_ORDER for i in DOWN_ORDER)
    first, issued = downs[0][0] + DOWN_LAG, 0
    for b, (jg, p) in enumerate(blocks):
        for jj in range(KD):
            for n, _ in enumerate(up(p, jg * KD + jj)):
                stage, k = 4 * (KD * b + jj) + n // 4, n % 4
                tick(8 * stage + 2 * k)
                goal = (4 * (stage - first) + k + 1) * 49 // (16 * KD)
                while downs and issued < goal and downs[0][0] <= stage:
                    downs.popleft()[1]()
                    issued += 1
                tick(8 * stage + 2 * k + 1)
    for _, work in downs:
        work()
        tick(None)
    while background:
        background.popleft()[1](token())
    wait(out_copy.values())


@jax.jit
def pallas_gated_mix__ssm_conv_h3__mixer_s_mlp__prompt_kernel(
    A_q: jax.Array,
    A_k: jax.Array,
    A_v: jax.Array,
    A_shift_k: jax.Array,
    A_ssm_k: jax.Array,
    A_ssm_D: jax.Array,
    B_x: jax.Array,
    B_w1: jax.Array,
    B_w2: jax.Array,
    B_w3: jax.Array,
    B_w4: jax.Array,
    gate_w: jax.Array,
):
    del B_x
    by_feature = lambda a: a.reshape(S, D).T
    hbm = pl.BlockSpec(memory_space=pl.ANY)
    scratch = (
        [pltpu.VMEM((KS, D), BF), pltpu.VMEM((D,), BF), pltpu.VMEM((D,), BF),
         pltpu.VMEM(_FWD.shape, I32), pltpu.VMEM(_INV.shape, I32)]
        + [pltpu.VMEM((D, S), BF)] * 4
        + [pltpu.VMEM((D, D), BF)] * 2
        + [pltpu.VMEM((D, F), BF)] * 2
        + [[pltpu.VMEM((49, Q, Q), BF)] * NP,
           [pltpu.VMEM((16, Q, DR), BF)] * NP,
           [pltpu.VMEM((49, Q, Q), BF)] * NJ,
           [pltpu.VMEM((16, DR, Q), BF)] * NJ,
           [pltpu.VMEM((49, DQ, Q), BF)] * NJ]
        + [pltpu.VMEM((KS + 2, D, Q), F32),
           pltpu.VMEM((D, S), F32),
           pltpu.VMEM((D, S), F32),
           pltpu.VMEM((8, S), F32),
           pltpu.VMEM((D, S), BF),
           pltpu.SemaphoreType.DMA((8,))]
    )
    out = pl.pallas_call(
        _kernel,
        in_specs=[hbm] * 13,
        out_specs=hbm,
        out_shape=jax.ShapeDtypeStruct((D, S), BF),
        scratch_shapes=scratch,
        compiler_params=pltpu.CompilerParams(
            vmem_limit_bytes=126 * 1024 * 1024,
            flags={'XLA_TPU_EVENLY_DISTRIBUTE_CRITICAL_NODES': True}),
    )(A_shift_k.T, A_ssm_D, gate_w, jnp.asarray(_FWD), jnp.asarray(_INV),
      by_feature(A_q), by_feature(A_k), by_feature(A_v), A_ssm_k, B_w1, B_w2, B_w3, B_w4.T)
    return out.T.reshape(1, S, D)
```

```python
import collections
import functools

import numpy as np
import jax
import jax.numpy as jnp
from jax import lax
import jax.experimental.pallas as pl
import jax.experimental.pallas.tpu as pltpu

BF = jnp.bfloat16
F32 = jnp.float32
I32 = jnp.int32

S, D, F = 2048, 576, 4608
KS = 4
Q = 128
NC = S // Q
TP = 4 * Q
NP = S // TP
FC = 4 * Q
NJ = F // FC
KD = 3
DQ = D // 4
DR = D - 4 * Q
TB = 2 * Q
NG = D // 8
EPS = 1e-5

_C0 = float(np.sqrt(2.0 / np.pi))
SC = float((_C0 * 0.044715) ** (1.0 / 3.0))
AA = _C0 / SC
UNSC = 0.5 / SC


def _bf16_words(a):
    u = a.astype(np.float32).view(np.uint32)
    u = (u + 0x7FFF + ((u >> 16) & 1)) >> 16
    return (u[0::2] | (u[1::2] << 16)).astype(np.uint32).view(np.int32)


def _transform_matrices():
    theta = 2.0 * np.pi * (np.arange(Q) + 0.25) / Q
    ang = np.arange(Q)[:, None] * theta[None, :]
    fwd = np.concatenate([np.cos(ang), -np.sin(ang)], axis=1)
    inv = np.concatenate([np.cos(ang).T, -np.sin(ang).T], axis=0) / Q
    return _bf16_words(fwd), _bf16_words(inv)


_FWD, _INV = _transform_matrices()
assert (_INV[0:8] != 0).all()


def _gelu(xs):
    return xs * (jnp.tanh(xs * (xs * xs + AA)) + 1.0)


def _layernorm(x):
    mean = jnp.sum(x, axis=0, keepdims=True) * (1.0 / D)
    xc = x - mean
    var = jnp.sum(xc * xc, axis=0, keepdims=True) * (1.0 / D)
    scale = lax.rsqrt(var + EPS) * SC
    return x * scale - mean * scale


K2 = ((0, 0), (0, 1), (1, 0), (1, 1))
WIDE = (0, 3, 4, 6)


LEFT = (((0, 0), 1, (1, 1)), ((1, 0), 1, (1, 1)), ((0, 0),), ((1, 1),),
        ((0, 0), 1, (0, 1)), ((1, 0), -1, (0, 0)), ((0, 1), -1, (1, 1)))
RIGHT = (((0, 0), 1, (1, 1)), ((0, 0),), ((0, 1), -1, (1, 1)), ((1, 0), -1, (0, 0)),
         ((1, 1),), ((0, 0), 1, (0, 1)), ((1, 0), 1, (1, 1)))


def _factor(rule, block):
    if len(rule) == 1:
        return block(rule[0])
    x, y = block(rule[0]), block(rule[2])
    return x + y if rule[1] > 0 else x - y


def _wide_a(a0, a1):
    return [a1, a1, a0, a0 - a1]


def _wide_b(b0, b1):
    return [b1, b0, b1, b0 + b1]


def _wide2(enc, quarters):
    outer = [enc(quarters[k], quarters[2 + k]) for k in range(2)]
    return [t for o in range(4) for t in enc(outer[0][o], outer[1][o])]


def _two(a, b):
    return a + b


def _four(a, b, c, d):
    return (a - b) + c + d


DECODE = (((0, 1), (2, 4), _two), ((1, 0), (1, 3), _two),
          ((0, 0), (3, 4, 0, 6), _four), ((1, 1), (2, 1, 0, 5), _four))


def _dec(m):
    return {blk: fn(*(m[i] for i in terms)) for blk, terms, fn in DECODE}


def _blockwise(fn, *ds):
    return {k: fn(*(d[k] for d in ds)) for k in K2}


STAGE_GROUPS = ((2, 4), (1, 3), (0, 6), (5,))
STAGE_ORDER = {
    1: ((0, 2), (0, 1), (0, 4), (0, 3), (0, 0), None, (0, 6), None, None, None, (0, 5)),
    2: ((0, 1), (0, 2), (0, 4), None, (0, 3), (1, 3), (1, 2), (1, 4), (1, 1), None,
        (0, 0), (0, 5), (0, 6), None, (1, 0), (1, 6), None, (1, 5)),
}
DOWN_ORDER = (1, 4, 0, 3, 6, 2, 5)
DOWN_READY = {1: 0, 0: 1, 4: 1, 3: 2, 6: 2, 2: 3, 5: 3}
DOWN_LAG = 4
HEAD = 'n2 n3 f2 n4 f3 n5 f4 f5 x0 s0 n6 s1 n7 s2 f6 f7 w0 s3 s4 s5 s6 s7'
MATMUL = 1000
MATMUL_TICKS = ((2, 6), (0, 4), (0, 4), (2, 6))
CONV_PAUSES = (1, 2, 2)
LAST_INPUTS_TICK = 183
RATES = dict(x=1.4, w=2.3, early=0.33, late=0.2)
MAX_CREDIT = 200


def _kernel(shift_hbm, ssmd_hbm, gate_hbm, fwd_hbm, inv_hbm,
            x_hbm, k_hbm, v_hbm, s_hbm, w1_hbm, w2_hbm, w3_hbm, w4_hbm,
            o_hbm,
            shift_ref, ssmd_ref, gate_ref, fwd_ref, inv_ref,
            kb, vb, sb, xb, w1b, w2b, w3b, w4b, xa, xr, w3a, w3r, w4a, coef, x1b, yb, gb, ob,
            sem):
    P = functools.partial

    def group(n, *parts):
        copies = []
        for src, dst, *window in parts:
            if window:
                at = tuple(pl.ds(lo, hi - lo) for lo, hi in window)
                src, dst = src.at[at], dst.at[at]
            copies.append(pltpu.make_async_copy(src, dst, sem.at[n]))
        return copies

    def start(copies):
        for c in copies:
            c.start()

    def wait(copies):
        for c in copies:
            c.wait()

    columns = lambda src, dst, lo, hi: (src, dst, (0, D), (lo, hi))
    inputs = [
        group(0, (shift_hbm, shift_ref), (ssmd_hbm, ssmd_ref), (gate_hbm, gate_ref)),
        group(1, columns(x_hbm, xb, 0, TB)),
        group(2, (w1_hbm, w1b), columns(x_hbm, xb, TB, 2 * TB)),
        group(3, (inv_hbm, inv_ref), columns(x_hbm, xb, 2 * TB, 6 * TB)),
        group(4, columns(x_hbm, xb, 6 * TB, S), (w2_hbm, w2b), columns(w3_hbm, w3b, 0, 2 * FC)),
        group(5, columns(w3_hbm, w3b, 2 * FC, KD * FC), columns(w4_hbm, w4b, 0, KD * FC)),
        group(6, columns(w3_hbm, w3b, KD * FC, F), columns(w4_hbm, w4b, KD * FC, F),
              (fwd_hbm, fwd_ref), (k_hbm, kb), (v_hbm, vb), (s_hbm, sb)),
    ]
    out_blocks = [(p, f, t) for p in range(NP) for f, t in K2]
    out_copy = dict(zip(out_blocks, group(7, *(
        (ob, o_hbm, (f * 2 * DQ, (f + 1) * 2 * DQ), (p * TP + t * 2 * Q, p * TP + (t + 1) * 2 * Q))
        for p, f, t in out_blocks))))

    last = [None]
    done = set()
    background = collections.deque()
    credit = dict(left=0.0, rate=0.0)

    def release(d):
        last[0] = d
        for r in range(0, d.shape[0], 32):
            credit['left'] = min(credit['left'] + 32 * credit['rate'] * (d.shape[1] // Q), MAX_CREDIT)
            while background and background[0][0] <= credit['left']:
                cost, work = background.popleft()
                credit['left'] -= cost
                work(d[r:r + 8, 0:Q])
        return d

    def dot(a, b):
        return release(jnp.dot(a, b, preferred_element_type=F32))

    def dot_nt(a, b):
        return release(lax.dot_general(a, b, (((1,), (1,)), ((), ())), preferred_element_type=F32))

    def token():
        return None if last[0] is None else last[0][0:8, 0:Q]

    def after(tok, x):
        if tok is None:
            return x
        if x.dtype == BF:
            return pltpu.bitcast(after(tok, pltpu.bitcast(x, I32)), BF)
        reps = (x.shape[0] // 8, x.shape[1] // Q)
        never = jnp.tile(inv_ref[0:8, :], reps) == 0
        return jnp.where(never, jnp.tile(pltpu.bitcast(tok, x.dtype), reps), x)

    def need(*what):
        while not done.issuperset(what):
            background.popleft()[1](token())

    lane = lax.broadcasted_iota(I32, (1, Q), 1)

    def operands(rules, load, buf, height):
        def piece(r, o, tok):
            def block(q, k):
                x = load(2 * q[0] + k[0], 2 * q[1] + k[1], r)
                return (after(tok, x) if q == rules[o][0] else x).astype(F32)
            outer = {k: _factor(rules[o], lambda q: block(q, k)) for k in K2}
            for i, rule in enumerate(rules):
                buf[7 * o + i, r:r + 16, :] = _factor(rule, outer.get).astype(BF)
        return [(50, P(piece, r, o)) for r in range(0, height, 16) for o in range(7)]

    def prepare_w3(j):
        cols = lambda h: slice(j * FC + h * Q, j * FC + (h + 1) * Q)

        def wide(tok):
            rest = [after(tok, w3b[4 * Q:D, cols(h)]).astype(F32) for h in range(4)]
            for i, t in enumerate(_wide2(_wide_b, rest)):
                w3r[j][i] = t.astype(BF)
            done.add(('w3', j))

        load = lambda k, h, r: w3b[k * Q + r:k * Q + r + 16, cols(h)]
        return operands(RIGHT, load, w3a[j], Q) + [(150, wide)]

    def prepare_w4(j):
        load = lambda f, k, r: w4b[f * DQ + r:f * DQ + r + 16, j * FC + (3 - k) * Q:j * FC + (4 - k) * Q]
        return operands(LEFT, load, w4a[j], DQ) + [(0, lambda tok: done.add(('w4', j)))]

    def prepare_x(p, quarters):
        def wide(r, tok):
            for i, t in enumerate(_wide2(_wide_a, [x[r:r + 64, 4 * Q:] for x in quarters])):
                xr[p][i, r:r + 64, :] = t.astype(BF)

        load = lambda t, k, r: quarters[t][r:r + 16, k * Q:(k + 1) * Q]
        return (operands(LEFT, load, xa[p], Q) + [(150, P(wide, r)) for r in range(0, Q, 64)]
                + [(0, lambda tok: done.add(('x', p)))])

    conv = {'left': NG}

    def conv_load(u):
        rows = slice(16 * u, 16 * u + 16)
        prev = [jnp.zeros((16, Q), F32)] * KS
        for c in range(NC):
            cols = slice(c * Q, (c + 1) * Q)
            kc = kb[rows, cols].astype(F32)
            cur = [kc] + [pltpu.roll(kc, t, 1) for t in range(1, KS)]
            ks = kc * coef[0, rows, :]
            for t in range(1, KS):
                ks = ks + jnp.where(lane >= t, cur[t], prev[t]) * coef[t, rows, :]
            prev = cur
            taps = sb[rows, cols].astype(F32)
            if c == 0:
                taps = taps + jnp.where(lane == 0, coef[KS, rows, :], 0.0)
            conv['in', u, c] = (ks * vb[rows, cols].astype(F32), taps)

    def causal(a, b):
        out = [a[0] * x for x in b]
        for m in range(1, NC):
            for c in range(m, NC):
                out[c] = out[c] + a[m] * b[c - m]
        return out

    def conv_forward(g, part, tok):
        if part == 0 and g % 2 == 0:
            conv_load(g // 2)
        half = slice(8 * (g % 2), 8 * (g % 2) + 8)
        rows = jnp.concatenate([conv['in', g // 2, c][part == 0][half] for c in range(NC)], axis=0)
        lo, hi = ((0, 2), (0, 1), (1, 2))[part]
        t = dot(rows.astype(BF), pltpu.bitcast(fwd_ref[:, lo * Q:hi * Q], BF))
        conv.setdefault(g, []).extend([t[8 * c:8 * c + 8, n * Q:(n + 1) * Q] for c in range(NC)]
                                      for n in range(hi - lo))
        if part < 2:
            return
        kr, ki, ur, ui = conv.pop(g)
        e, f = [y - x for x, y in zip(ur, ui)], [x + y for x, y in zip(ur, ui)]
        a = [kr[0]] + [kr[m] - ki[m - 1] for m in range(1, NC)]
        b = [ki[0]] + [ki[m] + kr[m - 1] for m in range(1, NC)]
        s1, s2, s3 = causal([x + y for x, y in zip(a, b)], ur), causal(a, e), causal(b, f)
        conv['z', g] = (jnp.concatenate([x - y for x, y in zip(s1, s3)], axis=0),
                        jnp.concatenate([x + y for x, y in zip(s1, s2)], axis=0))

    def conv_inverse(g, tok):
        y = dot(jnp.concatenate(conv.pop(('z', g)), axis=1).astype(BF), pltpu.bitcast(inv_ref[...], BF))
        for c in range(NC):
            yb[8 * g:8 * g + 8, c * Q:(c + 1) * Q] = y[8 * c:8 * c + 8]
        conv['left'] -= 1

    def conv_step(g):
        for part, pause in enumerate(CONV_PAUSES):
            if g < NG:
                yield MATMUL + part, P(conv_forward, g, part)
            yield from [(100, lambda tok: None)] * pause
        if g:
            yield MATMUL + 3, P(conv_inverse, g - 1)

    mix = {}
    zero = jnp.zeros((DQ, Q), F32)

    def mix_dot(w, x):
        return jnp.concatenate([dot(w[:D // 2], x), dot(w[D // 2:], x)], axis=0)

    def mix_norm(b):
        cols = slice(b * TB, (b + 1) * TB)
        x = after(token(), xb[:, cols]).astype(F32)
        mix['x', b] = _layernorm(x).astype(BF)
        z = jnp.sum(x * jnp.tile(coef[KS + 1], (1, TB // Q)), axis=0, keepdims=True)
        gb[:, cols] = jnp.broadcast_to(1.0 / (1.0 + jnp.exp(-z)), (8, TB))

    def mix_first(b):
        h = _gelu(mix_dot(mix['w1'], mix.pop(('x', b))))
        for i in range(TB // Q):
            mix['h', b * (TB // Q) + i] = [pltpu.roll(h[g * DQ:(g + 1) * DQ, i * Q:(i + 1) * Q], shift, 1)
                                           for g, shift in enumerate((1, Q - 1, 2, Q - 2))]

    def shifted(c):
        lo = mix['h', c - 1] if c > 0 else [zero] * 4
        hi = mix['h', c + 1] if c + 1 < NC else [zero] * 4
        cur = mix['h', c]
        return jnp.concatenate([jnp.where(lane >= 1, cur[0], lo[0]),
                                jnp.where(lane < Q - 1, cur[1], hi[1]),
                                jnp.where(lane >= 2, cur[2], lo[2]),
                                jnp.where(lane < Q - 2, cur[3], hi[3])], axis=0)

    def mix_second(b):
        cols, n = slice(b * TB, (b + 1) * TB), TB // Q
        hs = jnp.concatenate([shifted(b * n + i) for i in range(n)], axis=1).astype(BF)
        x1 = xb[:, cols].astype(F32) + mix_dot(mix['w2'], hs) * UNSC
        x1b[:, cols] = x1
        y = _layernorm(x1)
        for i in range(n):
            mix['y', b * n + i] = y[:, i * Q:(i + 1) * Q].T
        if (b + 1) * TB % TP == 0:
            p = (b + 1) * TB // TP - 1
            background.extendleft(reversed(prepare_x(p, [mix.pop(('y', 4 * p + t)) for t in range(4)])))

    hidden = {}
    out = {}

    def up(p, j):
        m, h = {}, {}
        for stage, groups in enumerate(STAGE_GROUPS):
            parts = {}
            for item in STAGE_ORDER[len(groups)]:
                if item is None:
                    yield
                    continue
                o, i = groups[item[0]], item[1]
                if o in WIDE and i in WIDE:
                    n = 4 * WIDE.index(o) + WIDE.index(i)
                    rest = dot(xr[p][n], w3r[j][n])
                    parts[o, i] = rest + dot(xa[p][7 * o + i], w3a[j][7 * o + i])
                else:
                    parts[o, i] = dot(xa[p][7 * o + i], w3a[j][7 * o + i])
            for o in groups:
                m[o] = _dec([parts[o, i] for i in range(7)])
            (t, c), terms, fn = DECODE[stage]
            h[1 - c, t] = _blockwise(lambda *v: _gelu(fn(*v)), *(m[o] for o in terms))
            for o in (o for o in range(7) if DOWN_READY[o] == stage):
                blk = {(k, n): _factor(RIGHT[o], lambda q: h[q][n, 1 - k]) for k, n in K2}
                for i, rule in enumerate(RIGHT):
                    hidden[p, j, 7 * o + i] = _factor(rule, blk.get).astype(BF)

    def finish(p, f, t, a, b, mlp, tok):
        rows = slice((2 * f + a) * DQ, (2 * f + a + 1) * DQ)
        cols = slice(p * TP + (2 * t + b) * Q, p * TP + (2 * t + b + 1) * Q)
        val = x1b[rows, cols] if mlp is None else x1b[rows, cols] + mlp * UNSC
        if conv['left']:
            x1b[rows, cols] = val
            background.append((100, P(finish, p, f, t, a, b, None)))
        else:
            h3 = after(tok, xb[rows, cols]).astype(F32) * yb[rows, cols]
            ob[rows, cols] = (val + gb[0:1, cols] * (h3 - val)).astype(BF)

    def down(p, jg, o, i):
        n, js = 7 * o + i, range(jg * KD, (jg + 1) * KD)
        need(*(('w4', j) for j in js))
        d0, d1, d2 = (dot_nt(w4a[j][n], hidden.pop((p, j, n))) for j in js)
        d = d0 + (d1 + d2)
        out[p, o, i] = out[p, o, i] + d if jg else d
        if jg < NJ // KD - 1 or i != DOWN_ORDER[-1]:
            return
        out[p, o] = _dec([out.pop((p, o, t)) for t in range(7)])
        for (f, t), terms, fn in DECODE:
            if o in terms and all((p, q) in out for q in terms):
                for (a, b), mlp in _blockwise(fn, *(out[p, q] for q in terms)).items():
                    finish(p, f, t, a, b, mlp, None)
                if conv['left']:
                    background.append((0, lambda tok, c=out_copy[p, f, t]: c.start()))
                else:
                    out_copy[p, f, t].start()

    start(inputs[0] + inputs[1] + inputs[2] + inputs[3])
    wait(inputs[0])
    taps = shift_ref[...].astype(F32)
    rows = [taps[t:t + 1] for t in range(KS)]
    rows += [r[...].astype(F32).reshape(1, D) for r in (ssmd_ref, gate_ref)]
    for i, r in enumerate(rows):
        coef[i] = jnp.broadcast_to(r, (Q, D)).T

    wait(inputs[1])
    mix_norm(0)
    wait(inputs[2])
    mix_norm(1)
    start(inputs[4] + inputs[5] + inputs[6])
    mix['w1'] = w1b[...].astype(F32).T.astype(BF)
    mix_first(0)
    mix_first(1)
    wait(inputs[3])
    last[0] = None
    for kind, b in HEAD.split():
        if kind == 'x':
            wait(inputs[4])
            background.extend(prepare_w3(0) + prepare_w3(1))
            mix['w2'] = w2b[...].astype(F32).T.astype(BF)
        elif kind == 'w':
            wait(inputs[5])
            background.extend(prepare_w3(2) + [w for j in range(KD) for w in prepare_w4(j)])
        else:
            dict(n=mix_norm, f=mix_first, s=mix_second)[kind](int(b))
            continue
        last[0] = None
        credit['rate'] = RATES[kind]
    credit['rate'] = RATES['early']

    def last_inputs():
        wait(inputs[6])
        credit['rate'] = RATES['late']
        weights = lambda jg: [w for prepare in (prepare_w3, prepare_w4)
                              for j in range(jg * KD, (jg + 1) * KD) for w in prepare(j)]
        background.extend(weights(1))
        for g in range(NG + 1):
            if g == NG // 3:
                background.extend(weights(2))
            background.extend(conv_step(g))

    def tick(n):
        if n == LAST_INPUTS_TICK:
            last_inputs()
        while background and background[0][0] >= MATMUL:
            if n is not None and n % 8 not in MATMUL_TICKS[background[0][0] - MATMUL]:
                break
            background.popleft()[1](None)

    blocks = [(jg, p) for jg in range(NJ // KD) for p in range(NP)]
    downs = collections.deque((4 * KD * (b + 1) - 3 + DOWN_READY[o], P(down, p, jg, o, i))
                              for b, (jg, p) in enumerate(blocks) for o in DOWN_ORDER for i in DOWN_ORDER)
    first, issued = downs[0][0] + DOWN_LAG, 0
    for b, (jg, p) in enumerate(blocks):
        for jj in range(KD):
            for n, _ in enumerate(up(p, jg * KD + jj)):
                stage, k = 4 * (KD * b + jj) + n // 4, n % 4
                tick(8 * stage + 2 * k)
                goal = (4 * (stage - first) + k + 1) * 49 // (16 * KD)
                while downs and issued < goal and downs[0][0] <= stage:
                    downs.popleft()[1]()
                    issued += 1
                tick(8 * stage + 2 * k + 1)
    for _, work in downs:
        work()
        tick(None)
    while background:
        background.popleft()[1](token())
    wait(out_copy.values())


@jax.jit
def pallas_gated_mix__ssm_conv_h3__mixer_s_mlp__prompt_kernel(
    A_q: jax.Array,
    A_k: jax.Array,
    A_v: jax.Array,
    A_shift_k: jax.Array,
    A_ssm_k: jax.Array,
    A_ssm_D: jax.Array,
    B_x: jax.Array,
    B_w1: jax.Array,
    B_w2: jax.Array,
    B_w3: jax.Array,
    B_w4: jax.Array,
    gate_w: jax.Array,
):
    del B_x
    by_feature = lambda a: a.reshape(S, D).T
    hbm = pl.BlockSpec(memory_space=pl.ANY)
    scratch = (
        [pltpu.VMEM((KS, D), BF), pltpu.VMEM((D,), BF), pltpu.VMEM((D,), BF),
         pltpu.VMEM(_FWD.shape, I32), pltpu.VMEM(_INV.shape, I32)]
        + [pltpu.VMEM((D, S), BF)] * 4
        + [pltpu.VMEM((D, D), BF)] * 2
        + [pltpu.VMEM((D, F), BF)] * 2
        + [[pltpu.VMEM((49, Q, Q), BF)] * NP,
           [pltpu.VMEM((16, Q, DR), BF)] * NP,
           [pltpu.VMEM((49, Q, Q), BF)] * NJ,
           [pltpu.VMEM((16, DR, Q), BF)] * NJ,
           [pltpu.VMEM((49, DQ, Q), BF)] * NJ]
        + [pltpu.VMEM((KS + 2, D, Q), F32),
           pltpu.VMEM((D, S), F32),
           pltpu.VMEM((D, S), F32),
           pltpu.VMEM((8, S), F32),
           pltpu.VMEM((D, S), BF),
           pltpu.SemaphoreType.DMA((8,))]
    )
    out = pl.pallas_call(
        _kernel,
        in_specs=[hbm] * 13,
        out_specs=hbm,
        out_shape=jax.ShapeDtypeStruct((D, S), BF),
        scratch_shapes=scratch,
        compiler_params=pltpu.CompilerParams(
            vmem_limit_bytes=126 * 1024 * 1024,
            flags={'XLA_TPU_EVENLY_DISTRIBUTE_CRITICAL_NODES': True}),
    )(A_shift_k.T, A_ssm_D, gate_w, jnp.asarray(_FWD), jnp.asarray(_INV),
      by_feature(A_q), by_feature(A_k), by_feature(A_v), A_ssm_k, B_w1, B_w2, B_w3, B_w4.T)
    return out.T.reshape(1, S, D)
```
